```python
import jax
import jax.numpy as jnp

def _softmax(x, axis=-1):
    return jax.nn.softmax(x, axis=axis)

def _gelu(x):
    return jax.nn.gelu(x, approximate=True)

def _silu(x):
    return jax.nn.silu(x)

def _sigmoid(x):
    return jax.nn.sigmoid(x)

def _layernorm(x, axis=-1, eps=1e-05):
    m = jnp.mean(x, axis=axis, keepdims=True)
    v = jnp.var(x, axis=axis, keepdims=True)
    return (x - m) / jnp.sqrt(v + eps)

def _scatter_add(tgt, idx, src, axis=0):
    return tgt.at[idx].add(src)

def _segment_sum(src, seg, n):
    return jax.ops.segment_sum(src, seg, n)

class _Rng:

    def __init__(self, key):
        self._k = key

    def _next(self):
        self._k, sub = jax.random.split(self._k)
        return sub

    def normal(self, shape):
        return jax.random.normal(self._next(), shape, dtype=jnp.bfloat16)

    def randint(self, lo, hi, shape):
        return jax.random.randint(self._next(), shape, lo, hi, dtype=jnp.int32)

    def uniform(self, shape, lo=0.0, hi=1.0):
        return jax.random.uniform(self._next(), shape, jnp.bfloat16, lo, hi)

    def permutation(self, n):
        return jax.random.permutation(self._next(), n)
kernel_name = 'interleave_layers__memory_aug_recurrent_mem_tr__glu_gated_geglu__prompt'

def setup_inputs():
    _rng = _Rng(jax.random.key(int.from_bytes(__import__("os").urandom(4), "little")))
    _w = lambda a: (lambda t: t.astype(jnp.bfloat16) if jnp.issubdtype(t.dtype, jnp.floating) else t)(jnp.asarray(a))

    def _A_setup():
        B, S, Dm = (1, 2048, 1024)
        H, Dh = (32, 128)
        M, seg = (8, 32)
        seg = min(seg, S)
        S = S // seg * seg
        return {'x': _w((lambda *s: _rng.normal(s) * 0.05)(B, S, Dm)), 'mem0': _w((lambda *s: _rng.normal(s) * 0.05)(B, M, Dm)), 'Wq': _w((lambda *s: _rng.normal(s) * 0.05)(Dm, H, Dh) * Dm ** (-0.5)), 'Wk': _w((lambda *s: _rng.normal(s) * 0.05)(Dm, H, Dh) * Dm ** (-0.5)), 'Wv': _w((lambda *s: _rng.normal(s) * 0.05)(Dm, H, Dh) * Dm ** (-0.5)), 'Wo': _w((lambda *s: _rng.normal(s) * 0.05)(H, Dh, Dm) * (H * Dh) ** (-0.5)), 'seg_len': seg}
    _A_in = _A_setup()

    def _B_setup():
        B, S, Dm, Df = (1, 2048, 1024, 3584)
        return {'x': _w((lambda *s: _rng.normal(s) * 0.05)(B, S, Dm)), 'w_gate': _w((lambda *s: _rng.normal(s) * 0.05)(Dm, Df) * Dm ** (-0.5)), 'w_up': _w((lambda *s: _rng.normal(s) * 0.05)(Dm, Df) * Dm ** (-0.5)), 'w_down': _w((lambda *s: _rng.normal(s) * 0.05)(Df, Dm) * Df ** (-0.5))}
    _B_in = _B_setup()
    return {'A_x': _A_in['x'], 'A_mem0': _A_in['mem0'], 'A_Wq': _A_in['Wq'], 'A_Wk': _A_in['Wk'], 'A_Wv': _A_in['Wv'], 'A_Wo': _A_in['Wo'], 'A_seg_len': _A_in['seg_len'], 'B_x': _B_in['x'], 'B_w_gate': _B_in['w_gate'], 'B_w_up': _B_in['w_up'], 'B_w_down': _B_in['w_down']}

def reference(A_x, A_mem0, A_Wq, A_Wk, A_Wv, A_Wo, A_seg_len, B_x, B_w_gate, B_w_up, B_w_down):

    def _A_ref(x, mem0, Wq, Wk, Wv, Wo, seg_len):
        B, S, Dm = x.shape
        H, Dh = (Wq.shape[1], Wq.shape[2])
        M = mem0.shape[1]
        scale = Dh ** (-0.5)
        n_seg = S // seg_len
        L = M + seg_len
        idx = jnp.arange(L)
        mask = (idx[:, None] < M) | (idx[:, None] >= idx[None, :])
        mem = mem0
        outs = []
        for s in range(n_seg):
            xs = x[:, s * seg_len:(s + 1) * seg_len, :].copy()
            h = jnp.concatenate([mem, xs], axis=1)
            q = jnp.einsum('btd,dhe->bhte', h, Wq)
            k = jnp.einsum('btd,dhe->bhte', h, Wk)
            v = jnp.einsum('btd,dhe->bhte', h, Wv)
            scores = jnp.einsum('bhqe,bhke->bhqk', q, k) * scale
            scores = jnp.where(mask[None, None], scores, -1000000000.0)
            p = _softmax(scores, axis=-1)
            o = jnp.einsum('bhqk,bhke->bhqe', p, v)
            o = jnp.einsum('bhte,hed->btd', o, Wo)
            mem = o[:, :M, :].copy()
            outs.append(o[:, M:, :])
        return jnp.concatenate(outs, axis=1)

    def _B_ref(x, w_gate, w_up, w_down):
        g = jnp.einsum('bsd,df->bsf', x, w_gate)
        u = jnp.einsum('bsd,df->bsf', x, w_up)
        h = _gelu(g) * u
        return jnp.einsum('bsf,fd->bsd', h, w_down)
    x = A_x
    x = x + _A_ref(_layernorm(x, axis=-1), A_mem0, A_Wq, A_Wk, A_Wv, A_Wo, A_seg_len)
    x = x + _B_ref(_layernorm(x, axis=-1), B_w_gate, B_w_up, B_w_down)
    x = x + _A_ref(_layernorm(x, axis=-1), A_mem0, A_Wq, A_Wk, A_Wv, A_Wo, A_seg_len)
    x = x + _B_ref(_layernorm(x, axis=-1), B_w_gate, B_w_up, B_w_down)
    return x
```

```python
import functools
import math

import jax
import jax.numpy as jnp
from jax import lax
import jax.experimental.pallas as pl
import jax.experimental.pallas.tpu as pltpu

_BF16 = jnp.bfloat16
_F32 = jnp.float32

_HG = 4
_FC = 512
_DCH = 128
_OUT_CH = 8


def _layernorm(x):
    m = jnp.mean(x, axis=-1, keepdims=True)
    c = x - m
    v = jnp.mean(c * c, axis=-1, keepdims=True)
    return c * lax.rsqrt(v + 1e-5)


def _gelu(x):
    k = math.sqrt(2.0 / math.pi)
    return x * (0.5 * (1.0 + jnp.tanh(k * (x + 0.044715 * (x * x * x)))))


def _dot(a, b):
    return jnp.dot(a, b, preferred_element_type=_F32)


def _full_order(n_g, n_f):
    b_ops = []
    for f in range(n_f):
        b_ops.append(("GU", f))
        if f >= 1:
            b_ops.append(("D", f - 1))
    b_ops.append(("D", n_f - 1))
    head = [b_ops[0], ("ZFIN", 0)]
    tail = b_ops[-2:]
    mid = b_ops[1:-2]
    order = list(head)
    slots = n_g + 1
    done = 0
    for g in range(n_g + 1):
        if g < n_g:
            order.append(("QKV", g))
        if g >= 1:
            order.append(("S", g - 1))
        if g >= 2:
            order.append(("O", g - 2))
        upto = (len(mid) * (g + 1)) // slots
        order.extend(mid[done:upto])
        done = upto
        if g >= 1:
            order.append(("PV", g - 1))
    order.append(tail[0])
    order.append(("O", n_g - 1))
    order.append(tail[1])
    order.append(("YFIN", 0))
    return order


def _attn_order(n_g):
    order = [("ZFIN", 0)]
    for g in range(n_g + 1):
        if g < n_g:
            order.append(("QKV", g))
        if g >= 1:
            order.append(("S", g - 1))
        if g >= 2:
            order.append(("O", g - 2))
        if g >= 1:
            order.append(("PV", g - 1))
    order.append(("O", n_g - 1))
    order.append(("YFIN", 0))
    return order


def _glu_order(n_f):
    order = [("GU", 0), ("ZOUT", 0)]
    for f in range(1, n_f):
        order.append(("GU", f))
        order.append(("D", f - 1))
    order.append(("D", n_f - 1))
    return order


def _kernel(x_hbm, mem0_ref, wq_hbm, wk_hbm, wv_hbm, wo_hbm, wg_hbm, wu_hbm, wd_hbm,
            out_hbm,
            stage, wqkv, wo, wg, wu, wd, xv, outv, ha, oacc, hb, rb, zacc, bias,
            sem_stage, sem_w, sem_out, *, n_heads, n_mem, seg):
    s_len, d_model = xv.shape
    d_ff = wg.shape[1]
    e = wo.shape[0] // n_heads
    n_seg = s_len // seg
    n_g = n_heads // _HG
    n_f = d_ff // _FC
    n_dch = d_model // _DCH
    m2 = 2 * n_mem
    rows = m2 + 2 * seg
    scale = e ** -0.5

    qkv_hbm = (wq_hbm, wk_hbm, wv_hbm)
    blk = _DCH // 16

    def stage_copy(w, c):
        return pltpu.make_async_copy(
            qkv_hbm[w].at[pl.ds(c * blk, blk)], stage.at[w, pl.ds(c * blk, blk)],
            sem_stage.at[w * n_dch + c])

    plain = ((x_hbm, xv), (wo_hbm, wo), (wg_hbm, wg), (wu_hbm, wu), (wd_hbm, wd))

    def plain_copy(i):
        return pltpu.make_async_copy(plain[i][0], plain[i][1], sem_w.at[i])

    plain_copy(0).start()
    for w in range(3):
        for c in range(n_dch):
            stage_copy(w, c).start()
    for i in range(1, len(plain)):
        plain_copy(i).start()

    r_id = lax.broadcasted_iota(jnp.int32, (rows, rows), 0)
    c_id = lax.broadcasted_iota(jnp.int32, (rows, rows), 1)

    def layer_of(i):
        return jnp.where(i < m2, i // n_mem, (i - m2) // seg)

    def pos_of(i):
        return jnp.where(i < m2, i % n_mem, n_mem + (i - m2) % seg)

    same = layer_of(r_id) == layer_of(c_id)
    keep = same & ((r_id < m2) | (pos_of(r_id) >= pos_of(c_id)))
    bias[...] = jnp.where(keep, 1.0, jnp.where(same, -1e9, -jnp.inf)).astype(_F32)

    mem0 = mem0_ref[...]
    ha[pl.ds(0, m2), :] = jnp.concatenate([mem0, mem0], axis=0).astype(_BF16)
    zacc[...] = jnp.zeros(zacc.shape, _F32)

    pairs = n_heads // 2
    for w in range(3):
        src = stage.at[w].bitcast(jnp.uint32)
        for c in range(n_dch):
            stage_copy(w, c).wait()

            def relayout(i, carry, src=src, w=w):
                d0 = pl.multiple_of(i * 16, 16)
                for j in range(pairs):
                    a = src[i, pl.ds(j, 8, stride=2 * pairs), :]
                    b = src[i, pl.ds(pairs + j, 8, stride=2 * pairs), :]
                    lo = (a & jnp.uint32(0xFFFF)) | (b << 16)
                    hi = (a >> 16) | (b & jnp.uint32(0xFFFF0000))
                    for h, val in ((2 * j, lo), (2 * j + 1, hi)):
                        col = (w * _HG + h % _HG) * e
                        wqkv[h // _HG, pl.ds(d0, 16), pl.ds(col, e)] = pltpu.bitcast(val, _BF16)
                return carry

            lax.fori_loop(c * blk, (c + 1) * blk, relayout, 0)

    def step(t, order):
        qkv, probs, att, hid = {}, {}, {}, {}

        def store_out(z2):
            so = jnp.clip(t - 4, 0, n_seg - 1)
            outv[pl.ds(pl.multiple_of(so * seg, seg), seg), :] = z2.astype(_BF16)

        for op, i in order:
            if op == "ZOUT":
                store_out(zacc[pl.ds(seg, seg), :])
            elif op == "ZFIN":
                z1 = zacc[pl.ds(0, seg), :]
                store_out(zacc[pl.ds(seg, seg), :])
                sx = jnp.minimum(t, n_seg - 1)
                xs = xv[pl.ds(pl.multiple_of(sx * seg, seg), seg), :].astype(_F32)
                ha[pl.ds(m2, seg), :] = _layernorm(xs).astype(_BF16)
                ha[pl.ds(m2 + seg, seg), :] = _layernorm(z1).astype(_BF16)
                oacc[pl.ds(0, m2), :] = jnp.zeros((m2, d_model), _F32)
                oacc[pl.ds(m2, seg), :] = xs
                oacc[pl.ds(m2 + seg, seg), :] = z1
            elif op == "QKV":
                qkv[i] = _dot(ha[...], wqkv[i]).astype(_BF16)
            elif op == "S":
                bv = bias[...]
                keep_m = bv > 0
                ps = []
                for h in range(_HG):
                    q = qkv[i][:, h * e:(h + 1) * e]
                    k = qkv[i][:, (_HG + h) * e:(_HG + h + 1) * e]
                    s = lax.dot_general(q, k, (((1,), (1,)), ((), ())),
                                        preferred_element_type=_F32)
                    s = jnp.where(keep_m, s * scale, bv)
                    p = jnp.exp(s - jnp.max(s, axis=-1, keepdims=True))
                    p = p / jnp.sum(p, axis=-1, keepdims=True)
                    ps.append(p.astype(_BF16))
                probs[i] = ps
            elif op == "PV":
                os_ = []
                for h in range(_HG):
                    v = qkv[i][:, (2 * _HG + h) * e:(2 * _HG + h + 1) * e]
                    os_.append(_dot(probs[i][h], v).astype(_BF16))
                att[i] = jnp.concatenate(os_, axis=1)
            elif op == "O":
                oacc[...] += _dot(att[i], wo[pl.ds(i * _HG * e, _HG * e), :])
            elif op == "YFIN":
                y = oacc[pl.ds(m2, 2 * seg), :]
                rb[...] = y
                hb[...] = _layernorm(y).astype(_BF16)
                mem2 = jnp.where(t >= 2, oacc[pl.ds(n_mem, n_mem), :],
                                 mem0_ref[...])
                ha[pl.ds(0, m2), :] = jnp.concatenate(
                    [oacc[pl.ds(0, n_mem), :], mem2], axis=0).astype(_BF16)
            elif op == "GU":
                hv = hb[...]
                g = _dot(hv, wg[:, pl.ds(i * _FC, _FC)])
                u = _dot(hv, wu[:, pl.ds(i * _FC, _FC)])
                hid[i] = (_gelu(g) * u).astype(_BF16)
            elif op == "D":
                part = _dot(hid[i], wd[pl.ds(i * _FC, _FC), :])
                if i == 0:
                    zacc[...] = rb[...] + part
                else:
                    zacc[...] += part

    def out_copy(c):
        n = _OUT_CH * seg
        return pltpu.make_async_copy(
            outv.at[pl.ds(c * n, n)], out_hbm.at[pl.ds(c * n, n)], sem_out.at[c])

    n_out = n_seg // _OUT_CH

    plain_copy(0).wait()
    plain_copy(1).wait()
    step(jnp.int32(0), _attn_order(n_g))
    for i in range(2, len(plain)):
        plain_copy(i).wait()

    full = _full_order(n_g, n_f)

    def body(t, carry):
        step(t, full)
        done = t - 3

        @pl.when((done >= _OUT_CH) & (done % _OUT_CH == 0))
        def _():
            out_copy(done // _OUT_CH - 1).start()

        return carry

    lax.fori_loop(1, n_seg + 2, body, 0)

    step(jnp.int32(n_seg + 2), _glu_order(n_f))
    outv[pl.ds((n_seg - 1) * seg, seg), :] = zacc[pl.ds(seg, seg), :].astype(_BF16)
    out_copy(n_out - 1).start()
    for c in range(n_out):
        out_copy(c).wait()


@jax.jit
def pallas_interleave_layers__memory_aug_recurrent_mem_tr__glu_gated_geglu__prompt_kernel(
    A_x: jax.Array,
    A_mem0: jax.Array,
    A_Wq: jax.Array,
    A_Wk: jax.Array,
    A_Wv: jax.Array,
    A_Wo: jax.Array,
    A_seg_len: jax.Array,
    B_x: jax.Array,
    B_w_gate: jax.Array,
    B_w_up: jax.Array,
    B_w_down: jax.Array,
):
    del B_x
    _, s_len, d_model = A_x.shape
    _, n_heads, e = A_Wq.shape
    n_mem = A_mem0.shape[1]
    d_ff = B_w_gate.shape[1]
    seg = A_seg_len if isinstance(A_seg_len, int) else min(32, s_len)
    rows = 2 * (n_mem + seg)
    n_g = n_heads // _HG

    def stage_view(w):
        return w.reshape(d_model // 16, 16 * n_heads, e)

    any_spec = pl.BlockSpec(memory_space=pl.ANY)
    out = pl.pallas_call(
        functools.partial(_kernel, n_heads=n_heads, n_mem=n_mem, seg=seg),
        out_shape=jax.ShapeDtypeStruct((s_len, d_model), _BF16),
        in_specs=[any_spec, pl.BlockSpec(memory_space=pltpu.VMEM)] + [any_spec] * 7,
        out_specs=any_spec,
        scratch_shapes=[
            pltpu.VMEM((3, d_model // 16, 16 * n_heads, e), _BF16),
            pltpu.VMEM((n_g, d_model, 3 * _HG * e), _BF16),
            pltpu.VMEM((n_heads * e, d_model), _BF16),
            pltpu.VMEM((d_model, d_ff), _BF16),
            pltpu.VMEM((d_model, d_ff), _BF16),
            pltpu.VMEM((d_ff, d_model), _BF16),
            pltpu.VMEM((s_len, d_model), _BF16),
            pltpu.VMEM((s_len, d_model), _BF16),
            pltpu.VMEM((rows, d_model), _BF16),
            pltpu.VMEM((rows, d_model), _F32),
            pltpu.VMEM((2 * seg, d_model), _BF16),
            pltpu.VMEM((2 * seg, d_model), _F32),
            pltpu.VMEM((2 * seg, d_model), _F32),
            pltpu.VMEM((rows, rows), _F32),
            pltpu.SemaphoreType.DMA((3 * (d_model // _DCH),)),
            pltpu.SemaphoreType.DMA((5,)),
            pltpu.SemaphoreType.DMA((s_len // seg // _OUT_CH,)),
        ],
        compiler_params=pltpu.CompilerParams(vmem_limit_bytes=110 * 1024 * 1024),
    )(
        A_x.reshape(s_len, d_model).astype(_BF16),
        A_mem0.reshape(n_mem, d_model).astype(_F32),
        stage_view(A_Wq).astype(_BF16), stage_view(A_Wk).astype(_BF16),
        stage_view(A_Wv).astype(_BF16),
        A_Wo.reshape(n_heads * e, d_model).astype(_BF16),
        B_w_gate.astype(_BF16), B_w_up.astype(_BF16), B_w_down.astype(_BF16),
    )
    return out.reshape(1, s_len, d_model).astype(A_x.dtype)
```

```python
import functools
import math

import jax
import jax.numpy as jnp
from jax import lax
import jax.experimental.pallas as pl
import jax.experimental.pallas.tpu as pltpu

_BF16 = jnp.bfloat16
_F32 = jnp.float32

_HG = 4
_FC = 256
_DCH = 128
_OUT_CH = 4
_LEAD = 3
_WINDOW = 3
_BURST = 28


def _layernorm(x):
    m = jnp.mean(x, axis=-1, keepdims=True)
    c = x - m
    v = jnp.mean(c * c, axis=-1, keepdims=True)
    return c * lax.rsqrt(v + 1e-5)


def _gelu(x):
    k = math.sqrt(2.0 / math.pi)
    return x * (0.5 * (1.0 + jnp.tanh(k * (x + 0.044715 * (x * x * x)))))


def _dot(a, b):
    return jnp.dot(a, b, preferred_element_type=_F32)


def _attn_order(n_g, fill=()):
    order = []
    done = 0
    for g in range(n_g + 1):
        if g < n_g:
            order.append(("QKV", g))
        if g == n_g:
            order.append(("NEXT", 0))
        if g >= 1:
            order.append(("S", g - 1))
        if g >= 2:
            order.append(("O", g - 2))
        upto = (len(fill) * (g + 1)) // (n_g + 1)
        order.extend(fill[done:upto])
        done = upto
        if g >= 1:
            order.append(("PV", g - 1))
    return order


def _glu_order(n_f):
    order = [("GU", 0)]
    for f in range(1, n_f):
        order.append(("GU", f))
        order.append(("D", f - 1))
    order.append(("D", n_f - 1))
    return order


def _full_order(n_g, n_f):
    glu = _glu_order(n_f)
    return ([glu[0]] + _attn_order(n_g, glu[1:-2])
            + [glu[-2], ("O", n_g - 1), ("YFIN", 0), glu[-1], ("ZFIN", 0)])


def _kernel(x_hbm, mem0_ref, wq_hbm, wk_hbm, wv_hbm, wo_hbm, wg_hbm, wu_hbm, wd_hbm,
            out_hbm,
            stage, wqkv, wo, wg, wu, wd, res, ha, oacc, hb, zacc, bias2, bias1,
            sem_stage, sem_x, sem_o, sem_f, sem_out, *, n_heads, n_mem, seg):
    s_len, d_model = res.shape
    d_ff = wg.shape[1]
    e = wo.shape[0] // n_heads
    n_seg = s_len // seg
    n_g = n_heads // _HG
    n_f = d_ff // _FC
    n_dch = d_model // _DCH
    m2 = 2 * n_mem
    scale = e ** -0.5

    qkv_hbm = (wq_hbm, wk_hbm, wv_hbm)
    blk = _DCH // 16
    x_head = (_LEAD + 1) * seg

    def x_copy(i):
        rows = pl.ds(0, x_head) if i == 0 else pl.ds(x_head, s_len - x_head)
        return pltpu.make_async_copy(x_hbm.at[rows], res.at[rows], sem_x.at[i])

    def stage_copy(w, c):
        return pltpu.make_async_copy(
            qkv_hbm[w].at[pl.ds(c * blk, blk)], stage.at[w, pl.ds(c * blk, blk)],
            sem_stage.at[w * n_dch + c])

    def wo_copy(g):
        rows = pl.ds(g * _HG * e, _HG * e)
        return pltpu.make_async_copy(wo_hbm.at[rows], wo.at[rows], sem_o.at[g])

    def glu_copy(w, f):
        cols = pl.ds(f * _FC, _FC)
        src, dst = ((wg_hbm.at[:, cols], wg.at[:, cols]),
                    (wu_hbm.at[:, cols], wu.at[:, cols]),
                    (wd_hbm.at[cols], wd.at[cols]))[w]
        return pltpu.make_async_copy(src, dst, sem_f.at[w * n_f + f])

    queue = [x_copy(0)]
    queue += [stage_copy(w, c) for w in range(3) for c in range(n_dch)]
    wo_at = len(queue)
    queue += [wo_copy(g) for g in range(n_g)]
    glu_at = {}
    for op, f in _glu_order(n_f):
        for w in ((0, 1) if op == "GU" else (2,)):
            glu_at[w, f] = len(queue)
            queue.append(glu_copy(w, f))
    queue.append(x_copy(1))
    issued = [0]

    def issue_upto(n):
        while issued[0] < min(n, len(queue)):
            queue[issued[0]].start()
            issued[0] += 1

    def arrive(i):
        issue_upto(i + 1)
        queue[i].wait()
        issue_upto(max(i + 1 + _WINDOW, issued[0] + 1))

    issue_upto(_WINDOW)

    def score_fill(n_rows, layer_of_token):
        r_id = lax.broadcasted_iota(jnp.int32, (n_rows, n_rows), 0)
        c_id = lax.broadcasted_iota(jnp.int32, (n_rows, n_rows), 1)

        def layer_of(i):
            return jnp.where(i < m2, i // n_mem, layer_of_token(i - m2))

        same = layer_of(r_id) == layer_of(c_id)
        keep = same & ((r_id < m2) | (r_id >= c_id))
        return jnp.where(keep, 1.0, jnp.where(same, -1e9, -jnp.inf)).astype(_F32)

    bias2[...] = score_fill(m2 + 2 * seg, lambda i: i // seg)
    for layer in range(2):
        bias1[layer] = score_fill(m2 + seg, lambda i, layer=layer: layer)

    arrive(0)
    mem0 = mem0_ref[...]
    ha[pl.ds(0, m2), :] = jnp.concatenate([mem0, mem0], axis=0).astype(_BF16)

    pairs = n_heads // 2
    for w in range(3):
        src = stage.at[w].bitcast(jnp.uint32)
        for c in range(n_dch):
            arrive(1 + w * n_dch + c)

            def relayout(i, carry, src=src, w=w):
                d0 = pl.multiple_of(i * 16, 16)
                for j in range(pairs):
                    a = src[i, pl.ds(j, 8, stride=2 * pairs), :]
                    b = src[i, pl.ds(pairs + j, 8, stride=2 * pairs), :]
                    lo = (a & jnp.uint32(0xFFFF)) | (b << 16)
                    hi = (a >> 16) | (b & jnp.uint32(0xFFFF0000))
                    for h, val in ((2 * j, lo), (2 * j + 1, hi)):
                        col = (w * _HG + h % _HG) * e
                        wqkv[h // _HG, pl.ds(d0, 16), pl.ds(col, e)] = pltpu.bitcast(val, _BF16)
                return carry

            lax.fori_loop(c * blk, (c + 1) * blk, relayout, 0)

    def rows_of(s):
        return pl.ds(pl.multiple_of(s * seg, seg), seg)

    def load_segs(segs):
        return jnp.concatenate([res[rows_of(s), :] for s in segs], axis=0).astype(_F32)

    def store_segs(segs, val):
        for i, s in enumerate(segs):
            res[rows_of(s), :] = val[i * seg:(i + 1) * seg]

    def prep_attn(segs):
        ha[pl.ds(m2, len(segs) * seg), :] = _layernorm(load_segs(segs)).astype(_BF16)

    def prep_glu(segs):
        hb[pl.ds(0, len(segs) * seg), :] = _layernorm(load_segs(segs)).astype(_BF16)

    def run(order, a_segs=(), b_segs=(), layer=None, next_a=None, streaming=False):
        a_rows = m2 + len(a_segs) * seg
        b_rows = len(b_segs) * seg
        qkv, probs, att, hid = {}, {}, {}, {}
        for op, i in order:
            if op == "QKV":
                qkv[i] = _dot(ha[pl.ds(0, a_rows), :], wqkv[i]).astype(_BF16)
            elif op == "NEXT":
                if next_a is not None:
                    prep_attn(next_a)
            elif op == "S":
                fill = bias2[...] if layer is None else bias1[layer]
                keep = fill > 0
                ps = []
                for h in range(_HG):
                    q = qkv[i][:, h * e:(h + 1) * e]
                    k = qkv[i][:, (_HG + h) * e:(_HG + h + 1) * e]
                    s = lax.dot_general(q, k, (((1,), (1,)), ((), ())),
                                        preferred_element_type=_F32)
                    s = jnp.where(keep, s * scale, fill)
                    p = jnp.exp(s - jnp.max(s, axis=-1, keepdims=True))
                    p = p / jnp.sum(p, axis=-1, keepdims=True)
                    ps.append(p.astype(_BF16))
                probs[i] = ps
            elif op == "PV":
                heads = []
                for h in range(_HG):
                    v = qkv[i][:, (2 * _HG + h) * e:(2 * _HG + h + 1) * e]
                    heads.append(_dot(probs[i][h], v).astype(_BF16))
                att[i] = jnp.concatenate(heads, axis=1)
            elif op == "O":
                if streaming:
                    arrive(wo_at + i)
                part = _dot(att[i], wo[pl.ds(i * _HG * e, _HG * e), :])
                if i == 0:
                    oacc[pl.ds(0, m2), :] = part[:m2]
                    oacc[pl.ds(m2, a_rows - m2), :] = load_segs(a_segs) + part[m2:]
                else:
                    oacc[pl.ds(0, a_rows), :] += part
            elif op == "YFIN":
                y = oacc[pl.ds(m2, a_rows - m2), :].astype(_BF16)
                store_segs(a_segs, y)
                mem = oacc[pl.ds(0, m2), :]
                if layer is None:
                    hb[pl.ds(0, a_rows - m2), :] = _layernorm(y.astype(_F32)).astype(_BF16)
                else:
                    row = lax.broadcasted_iota(jnp.int32, mem.shape, 0)
                    mine = (row >= layer * n_mem) & (row < (layer + 1) * n_mem)
                    mem = jnp.where(mine, mem, ha[pl.ds(0, m2), :].astype(_F32))
                ha[pl.ds(0, m2), :] = mem.astype(_BF16)
            elif op == "GU":
                if streaming:
                    arrive(glu_at[0, i])
                    arrive(glu_at[1, i])
                hv = hb[pl.ds(0, b_rows), :]
                g = _dot(hv, wg[:, pl.ds(i * _FC, _FC)])
                u = _dot(hv, wu[:, pl.ds(i * _FC, _FC)])
                hid[i] = (_gelu(g) * u).astype(_BF16)
            elif op == "D":
                if streaming:
                    arrive(glu_at[2, i])
                part = _dot(hid[i], wd[pl.ds(i * _FC, _FC), :])
                if i == 0:
                    zacc[pl.ds(0, b_rows), :] = load_segs(b_segs) + part
                else:
                    zacc[pl.ds(0, b_rows), :] += part
            elif op == "ZFIN":
                store_segs(b_segs, zacc[pl.ds(0, b_rows), :].astype(_BF16))

    def attn_only(layer, s, streaming=False):
        prep_attn([s])
        run(_attn_order(n_g) + [("O", n_g - 1), ("YFIN", 0)], a_segs=[s], layer=layer,
            streaming=streaming)

    def glu_only(segs, streaming=False):
        prep_glu(segs)
        run(_glu_order(n_f) + [("ZFIN", 0)], b_segs=segs, streaming=streaming)

    def loop(lo, hi, fn):
        def body(i, carry):
            fn(i)
            return carry
        lax.fori_loop(lo, hi, body, 0)

    def out_copy(c):
        n = _OUT_CH * seg
        return pltpu.make_async_copy(
            res.at[pl.ds(c * n, n)], out_hbm.at[pl.ds(c * n, n)], sem_out.at[c])

    n_out = n_seg // _OUT_CH
    n_main = n_seg - _LEAD

    attn_only(jnp.int32(0), 0, streaming=True)
    issue_upto(glu_at[0, 0] + _BURST)
    loop(1, _LEAD, lambda s: attn_only(jnp.int32(0), s))
    glu_only(list(range(_LEAD)), streaming=True)
    loop(0, 2, lambda layer: attn_only(layer, _LEAD * (1 - layer)))
    arrive(len(queue) - 1)
    prep_attn([_LEAD + 1, 1])
    prep_glu([_LEAD, 0])

    full = _full_order(n_g, n_f)

    def full_step(j):
        run(full, a_segs=[j + _LEAD, j], b_segs=[j + _LEAD - 1, j - 1],
            next_a=[jnp.minimum(j + _LEAD + 1, n_seg - 1), j + 1])

        @pl.when(j % _OUT_CH == 0)
        def _():
            out_copy(j // _OUT_CH - 1).start()

    loop(1, n_main, full_step)

    run(_glu_order(n_f) + [("ZFIN", 0)], b_segs=[n_seg - 1, n_main - 1])
    started = (n_main - 1) // _OUT_CH
    for c in range(started, n_main // _OUT_CH):
        out_copy(c).start()
    loop(n_main, n_seg, lambda s: attn_only(jnp.int32(1), s))
    glu_only(list(range(n_main, n_seg)))
    for c in range(n_main // _OUT_CH, n_out):
        out_copy(c).start()
    for c in range(n_out):
        out_copy(c).wait()


@jax.jit
def pallas_interleave_layers__memory_aug_recurrent_mem_tr__glu_gated_geglu__prompt_kernel(
    A_x: jax.Array,
    A_mem0: jax.Array,
    A_Wq: jax.Array,
    A_Wk: jax.Array,
    A_Wv: jax.Array,
    A_Wo: jax.Array,
    A_seg_len: jax.Array,
    B_x: jax.Array,
    B_w_gate: jax.Array,
    B_w_up: jax.Array,
    B_w_down: jax.Array,
):
    del B_x
    _, s_len, d_model = A_x.shape
    _, n_heads, e = A_Wq.shape
    n_mem = A_mem0.shape[1]
    d_ff = B_w_gate.shape[1]
    seg = A_seg_len if isinstance(A_seg_len, int) else min(32, s_len)
    rows = 2 * (n_mem + seg)
    n_g = n_heads // _HG

    def stage_view(w):
        return w.reshape(d_model // 16, 16 * n_heads, e)

    any_spec = pl.BlockSpec(memory_space=pl.ANY)
    out = pl.pallas_call(
        functools.partial(_kernel, n_heads=n_heads, n_mem=n_mem, seg=seg),
        out_shape=jax.ShapeDtypeStruct((s_len, d_model), _BF16),
        in_specs=[any_spec, pl.BlockSpec(memory_space=pltpu.VMEM)] + [any_spec] * 7,
        out_specs=any_spec,
        scratch_shapes=[
            pltpu.VMEM((3, d_model // 16, 16 * n_heads, e), _BF16),
            pltpu.VMEM((n_g, d_model, 3 * _HG * e), _BF16),
            pltpu.VMEM((n_heads * e, d_model), _BF16),
            pltpu.VMEM((d_model, d_ff), _BF16),
            pltpu.VMEM((d_model, d_ff), _BF16),
            pltpu.VMEM((d_ff, d_model), _BF16),
            pltpu.VMEM((s_len, d_model), _BF16),
            pltpu.VMEM((rows, d_model), _BF16),
            pltpu.VMEM((rows, d_model), _F32),
            pltpu.VMEM((_LEAD * seg, d_model), _BF16),
            pltpu.VMEM((_LEAD * seg, d_model), _F32),
            pltpu.VMEM((rows, rows), _F32),
            pltpu.VMEM((2, rows - seg, rows - seg), _F32),
            pltpu.SemaphoreType.DMA((3 * (d_model // _DCH),)),
            pltpu.SemaphoreType.DMA((2,)),
            pltpu.SemaphoreType.DMA((n_g,)),
            pltpu.SemaphoreType.DMA((3 * (d_ff // _FC),)),
            pltpu.SemaphoreType.DMA((s_len // seg // _OUT_CH,)),
        ],
        compiler_params=pltpu.CompilerParams(vmem_limit_bytes=110 * 1024 * 1024),
    )(
        A_x.reshape(s_len, d_model).astype(_BF16),
        A_mem0.reshape(n_mem, d_model).astype(_F32),
        stage_view(A_Wq).astype(_BF16), stage_view(A_Wk).astype(_BF16),
        stage_view(A_Wv).astype(_BF16),
        A_Wo.reshape(n_heads * e, d_model).astype(_BF16),
        B_w_gate.astype(_BF16), B_w_up.astype(_BF16), B_w_down.astype(_BF16),
    )
    return out.reshape(1, s_len, d_model).astype(A_x.dtype)
```

```python
import functools
import math

import jax
import jax.numpy as jnp
from jax import lax
import jax.experimental.pallas as pl
import jax.experimental.pallas.tpu as pltpu

_BF16 = jnp.bfloat16
_F32 = jnp.float32

_HG = 4
_T = 128
_DCH = 128
_OUT_CH = 4
_LEAD = 4
_WINDOW = 3
_D_BATCH = 2


def _layernorm(x):
    m = jnp.mean(x, axis=-1, keepdims=True)
    c = x - m
    v = jnp.mean(c * c, axis=-1, keepdims=True)
    return c * lax.rsqrt(v + 1e-5)


def _gelu(x):
    k = math.sqrt(2.0 / math.pi)
    return x * (0.5 * (1.0 + jnp.tanh(k * (x + 0.044715 * (x * x * x)))))


def _dot(a, b):
    return jnp.dot(a, b, preferred_element_type=_F32)


def _lhs_blocks(a11, a12, a21, a22):
    return (a11 + a22, a21 + a22, a11, a22, a11 + a12, a21 - a11, a12 - a22)


def _rhs_blocks(b11, b12, b21, b22):
    return (b11 + b22, b11, b12 - b22, b21 - b11, b22, b11 + b12, b21 + b22)


def _out_blocks(m1, m2, m3, m4, m5, m6, m7):
    return (m1 + m4 - m5 + m7, m3 + m5, m2 + m4, m1 - m2 + m3 + m6)


def _attn_order(n_g, fill=()):
    order = []
    done = 0
    for g in range(n_g + 1):
        if g < n_g:
            order.append(("QKV", g))
        if g >= 1:
            order.append(("S", g - 1))
        if g >= 2:
            order.append(("O", g - 2))
        upto = (len(fill) * (g + 1)) // (n_g + 1)
        order.extend(fill[done:upto])
        done = upto
        if g >= 1:
            order.append(("PV", g - 1))
    return order


def _glu_order(n_c):
    order = []
    start = 0
    for c in range(n_c):
        order.append(("GU", c))
        if c - start == _D_BATCH and c < n_c - 1:
            order.append(("D", (start, c)))
            start = c
    if n_c - start > 1:
        order.append(("D", (start, n_c - 1)))
    order.append(("D", (n_c - 1, n_c)))
    return order


def _full_order(n_g, n_c):
    glu = _glu_order(n_c)
    return ([glu[0], ("ZFIN", 0)] + _attn_order(n_g, glu[1:-2])
            + [glu[-2], ("O", n_g - 1), ("YFIN", 0), glu[-1]])


def _kernel(x_hbm, mem0_ref, wq_hbm, wk_hbm, wv_hbm, wo_hbm, wg_hbm, wu_hbm, wd_hbm,
            out_hbm,
            wqkv, wo, wgu, wd, res, ha, oacc, hb, macc, bias2, bias1,
            sem_stage, sem_x, sem_o, sem_f, sem_out, *, n_heads, n_mem, seg):
    s_len, d_model = x_hbm.shape
    d_ff = wg_hbm.shape[1]
    e = wo.shape[0] // n_heads
    n_seg = s_len // seg
    n_g = n_heads // _HG
    n_chunks = d_ff // (2 * _T)
    n_c = n_chunks // 2
    n_dch = d_model // _DCH
    half = d_model // 2
    m2 = 2 * n_mem
    scale = e ** -0.5
    spare = n_seg

    queue = []
    issued = [0]

    def issue_upto(n):
        while issued[0] < min(n, len(queue)):
            queue[issued[0]]().start()
            issued[0] += 1

    def arrive(i):
        issue_upto(i + 1)
        queue[i]().wait()
        issue_upto(i + 1 + _WINDOW)

    x_head = (_LEAD + 2) * seg

    def x_copy(i):
        rows = pl.ds(0, x_head) if i == 0 else pl.ds(x_head, s_len - x_head)
        return pltpu.make_async_copy(x_hbm.at[rows], res.at[rows], sem_x.at[i])

    def wo_copy(g):
        rows = pl.ds(g * _HG * e, _HG * e)
        return pltpu.make_async_copy(wo_hbm.at[rows], wo.at[rows], sem_o.at[g])

    def load_attention_weights(stage):
        blk = _DCH // 16

        def stage_copy(w, c):
            return pltpu.make_async_copy(
                (wq_hbm, wk_hbm, wv_hbm)[w].at[pl.ds(c * blk, blk)],
                stage.at[w, pl.ds(c * blk, blk)], sem_stage.at[w * n_dch + c])

        queue.append(functools.partial(x_copy, 0))
        queue.extend(functools.partial(stage_copy, w, c)
                     for w in range(3) for c in range(n_dch))
        queue.extend(functools.partial(wo_copy, g) for g in range(n_g))
        issue_upto(_WINDOW)

        def score_fill(n_rows, layer_of_token):
            r_id = lax.broadcasted_iota(jnp.int32, (n_rows, n_rows), 0)
            c_id = lax.broadcasted_iota(jnp.int32, (n_rows, n_rows), 1)

            def layer_of(i):
                return jnp.where(i < m2, i // n_mem, layer_of_token(i - m2))

            same = layer_of(r_id) == layer_of(c_id)
            keep = same & ((r_id < m2) | (r_id >= c_id))
            return jnp.where(keep, 1.0, jnp.where(same, -1e9, -jnp.inf)).astype(_F32)

        bias2[...] = score_fill(m2 + 2 * seg, lambda i: i // seg)
        for layer in range(2):
            bias1[layer] = score_fill(m2 + seg, lambda i, layer=layer: layer)
        res[pl.ds(spare * seg, seg), :] = jnp.zeros((seg, d_model), _BF16)
        arrive(0)
        mem0 = mem0_ref[...]
        ha[pl.ds(0, m2), :] = jnp.concatenate([mem0, mem0], axis=0).astype(_BF16)

        pairs = n_heads // 2
        for w in range(3):
            src = stage.at[w].bitcast(jnp.uint32)
            for c in range(n_dch):
                arrive(1 + w * n_dch + c)

                def relayout(i, carry, src=src, w=w):
                    d0 = pl.multiple_of(i * 16, 16)
                    for j in range(pairs):
                        a = src[i, pl.ds(j, 8, stride=2 * pairs), :]
                        b = src[i, pl.ds(pairs + j, 8, stride=2 * pairs), :]
                        lo = (a & jnp.uint32(0xFFFF)) | (b << 16)
                        hi = (a >> 16) | (b & jnp.uint32(0xFFFF0000))
                        for h, val in ((2 * j, lo), (2 * j + 1, hi)):
                            col = (w * _HG + h % _HG) * e
                            wqkv[h // _HG, pl.ds(d0, 16), pl.ds(col, e)] = (
                                pltpu.bitcast(val, _BF16))
                    return carry

                lax.fori_loop(c * blk, (c + 1) * blk, relayout, 0)

    pl.run_scoped(load_attention_weights,
                  pltpu.VMEM((3, d_model // 16, 16 * n_heads, e), _BF16))
    wo_at = 1 + 3 * n_dch

    def rows_of(s):
        if isinstance(s, int):
            return pl.ds(s * seg, seg)
        return pl.ds(pl.multiple_of(s * seg, seg), seg)

    def load_segs(segs):
        return jnp.concatenate([res[rows_of(s), :] for s in segs], axis=0).astype(_F32)

    def prep_attn(vals):
        ha[pl.ds(m2, vals.shape[0]), :] = _layernorm(vals).astype(_BF16)

    def prep_glu(buf, part, vals):
        h = _layernorm(vals)
        blocks = _lhs_blocks(h[:seg, :half], h[:seg, half:], h[seg:, :half], h[seg:, half:])
        for i, blk in enumerate(blocks):
            hb[buf, i, rows_of(part), :] = blk.astype(_BF16)

    def finish_glu(buf, part, top, bottom):
        c11, c12, c21, c22 = _out_blocks(*(macc[buf, i, rows_of(part), :] for i in range(7)))
        z_top = (load_segs([top]) + jnp.concatenate([c11, c12], axis=1)).astype(_BF16)
        z_bot = (load_segs([bottom]) + jnp.concatenate([c21, c22], axis=1)).astype(_BF16)
        res[rows_of(top), :] = z_top
        res[rows_of(bottom), :] = z_bot
        return z_top

    def run(order, step=None, a_segs=(), layer=None, streaming=False):
        a_rows = m2 + len(a_segs) * seg
        if step is not None:
            part = step % 2
            buf = (step // 2) % 2
        qkv, probs, att, hid = {}, {}, {}, {}
        for op, i in order:
            if op == "ZFIN":
                done = jnp.where(step >= _LEAD, step - _LEAD, spare)
                z1 = finish_glu(1 - buf, part, step, done)
                prep_attn(jnp.concatenate(
                    [load_segs(a_segs[:1]), z1.astype(_F32)], axis=0))
            elif op == "QKV":
                qkv[i] = _dot(ha[pl.ds(0, a_rows), :], wqkv[i]).astype(_BF16)
            elif op == "S":
                fill = bias2[...] if layer is None else bias1[layer]
                keep = fill > 0
                ps = []
                for h in range(_HG):
                    q = qkv[i][:, h * e:(h + 1) * e]
                    k = qkv[i][:, (_HG + h) * e:(_HG + h + 1) * e]
                    s = lax.dot_general(q, k, (((1,), (1,)), ((), ())),
                                        preferred_element_type=_F32)
                    s = jnp.where(keep, s * scale, fill)
                    p = jnp.exp(s - jnp.max(s, axis=-1, keepdims=True))
                    p = p / jnp.sum(p, axis=-1, keepdims=True)
                    ps.append(p.astype(_BF16))
                probs[i] = ps
            elif op == "PV":
                heads = []
                for h in range(_HG):
                    v = qkv[i][:, (2 * _HG + h) * e:(2 * _HG + h + 1) * e]
                    heads.append(_dot(probs[i][h], v).astype(_BF16))
                att[i] = jnp.concatenate(heads, axis=1)
            elif op == "O":
                if streaming:
                    arrive(wo_at + i)
                out = _dot(att[i], wo[pl.ds(i * _HG * e, _HG * e), :])
                if i == 0:
                    oacc[pl.ds(0, m2), :] = out[:m2]
                    oacc[pl.ds(m2, a_rows - m2), :] = load_segs(a_segs) + out[m2:]
                else:
                    oacc[pl.ds(0, a_rows), :] += out
            elif op == "YFIN":
                y = oacc[pl.ds(m2, a_rows - m2), :].astype(_BF16)
                for k, s in enumerate(a_segs):
                    res[rows_of(s), :] = y[k * seg:(k + 1) * seg]
                mem = oacc[pl.ds(0, m2), :]
                if layer is None:
                    prep_glu(1 - buf, part, y.astype(_F32))
                else:
                    row = lax.broadcasted_iota(jnp.int32, mem.shape, 0)
                    mine = (row >= layer * n_mem) & (row < (layer + 1) * n_mem)
                    mem = jnp.where(mine, mem, ha[pl.ds(0, m2), :].astype(_F32))
                ha[pl.ds(0, m2), :] = mem.astype(_BF16)
            elif op == "GU":
                c = part * n_c + i
                c11, c12, c21, c22 = _out_blocks(
                    *(_dot(hb[buf, k], wgu[k, c]) for k in range(7)))
                hid[i] = [blk.astype(_BF16) for blk in _lhs_blocks(
                    *(_gelu(blk[:, :_T]) * blk[:, _T:] for blk in (c11, c12, c21, c22)))]
            elif op == "D":
                lo, hi = i
                rows = pl.ds(pl.multiple_of((part * n_c + lo) * _T, _T), (hi - lo) * _T)
                for k in range(7):
                    lhs = jnp.concatenate([hid[c][k] for c in range(lo, hi)], axis=1)
                    out = _dot(lhs, wd[k, rows, :])
                    if lo == 0:
                        macc[buf, k] = jnp.where(part == 0, out, macc[buf, k] + out)
                    else:
                        macc[buf, k] += out

    def loop(lo, hi, fn):
        def body(i, carry):
            fn(i)
            return carry
        lax.fori_loop(lo, hi, body, 0)

    attn_all = _attn_order(n_g) + [("O", n_g - 1), ("YFIN", 0)]

    def attn_one(layer, s, streaming=False):
        prep_attn(load_segs([s]))
        run(attn_all, a_segs=[s], layer=layer, streaming=streaming)

    def glu_four(buf, first):
        loop(0, 2, lambda part: prep_glu(
            buf, part, load_segs([first + 2 + part, first + part])))
        loop(2 * buf, 2 * buf + 2, lambda step: run(_glu_order(n_c), step=step))

    def head_start(raw_g, raw_u, raw_d):
        def raw_copy(w, c):
            start = c * 2 * _T
            cols = pl.ds(start if isinstance(c, int) else pl.multiple_of(start, 2 * _T), 2 * _T)
            src, dst = ((wg_hbm.at[:, cols], raw_g.at[c]), (wu_hbm.at[:, cols], raw_u.at[c]),
                        (wd_hbm.at[cols], raw_d.at[c]))[w]
            return pltpu.make_async_copy(src, dst, sem_f.at[w, c])

        def split_weights(c):
            for w in range(3):
                raw_copy(w, c).wait()
            for w, raw in enumerate((raw_g, raw_u)):
                quads = (raw[c, pl.ds(r, half), pl.ds(k, _T)].astype(_F32)
                         for r in (0, half) for k in (0, _T))
                for i, blk in enumerate(_rhs_blocks(*quads)):
                    wgu[i, c, :, pl.ds(w * _T, _T)] = blk.astype(_BF16)
            quads = (raw_d[c, pl.ds(r, _T), pl.ds(k, half)].astype(_F32)
                     for r in (0, _T) for k in (0, half))
            for i, blk in enumerate(_rhs_blocks(*quads)):
                wd[i, pl.ds(pl.multiple_of(c * _T, _T), _T), :] = blk.astype(_BF16)

        attn_one(0, 0, streaming=True)
        for c in range(n_chunks):
            for w in range(3):
                raw_copy(w, c).start()
        loop(1, _LEAD, lambda s: attn_one(0, s))
        x_copy(1).start()
        loop(0, n_chunks, split_weights)

    pl.run_scoped(head_start,
                  pltpu.VMEM((n_chunks, d_model, 2 * _T), _BF16),
                  pltpu.VMEM((n_chunks, d_model, 2 * _T), _BF16),
                  pltpu.VMEM((n_chunks, 2 * _T, d_model), _BF16))

    macc[...] = jnp.zeros(macc.shape, _F32)
    glu_four(0, 0)
    loop(0, 2, lambda part: finish_glu(0, part, spare, part))
    x_copy(1).wait()

    def attn_step(j):
        segs = [j + _LEAD, j]
        prep_attn(load_segs(segs))
        run(attn_all, step=j, a_segs=segs)

    loop(0, 2, attn_step)

    def out_copy(c):
        n = _OUT_CH * seg
        return pltpu.make_async_copy(
            res.at[pl.ds(c * n, n)], out_hbm.at[pl.ds(c * n, n)], sem_out.at[c])

    n_out = n_seg // _OUT_CH
    n_main = n_seg - _LEAD
    full = _full_order(n_g, n_c)

    def full_step(j):
        run(full, step=j, a_segs=[j + _LEAD, j])
        final = j + 1 - _LEAD

        @pl.when((final > 0) & (final % _OUT_CH == 0))
        def _():
            out_copy(final // _OUT_CH - 1).start()

    loop(2, n_main, full_step)

    buf = (n_main // 2) % 2
    loop(0, 2, lambda part: finish_glu(
        1 - buf, part, n_main + part, n_main - _LEAD + part))
    loop(2 * buf, 2 * buf + 2, lambda step: run(_glu_order(n_c), step=step))
    loop(0, 2, lambda part: finish_glu(
        buf, part, n_main + 2 + part, n_main - 2 + part))
    out_copy(n_out - 2).start()
    loop(n_main, n_seg, lambda s: attn_one(1, s))
    glu_four(0, n_main)
    loop(0, 2, lambda part: finish_glu(0, part, n_main + 2 + part, n_main + part))
    out_copy(n_out - 1).start()
    for c in range(n_out):
        out_copy(c).wait()


@jax.jit
def pallas_interleave_layers__memory_aug_recurrent_mem_tr__glu_gated_geglu__prompt_kernel(
    A_x: jax.Array,
    A_mem0: jax.Array,
    A_Wq: jax.Array,
    A_Wk: jax.Array,
    A_Wv: jax.Array,
    A_Wo: jax.Array,
    A_seg_len: jax.Array,
    B_x: jax.Array,
    B_w_gate: jax.Array,
    B_w_up: jax.Array,
    B_w_down: jax.Array,
):
    del B_x
    _, s_len, d_model = A_x.shape
    _, n_heads, e = A_Wq.shape
    n_mem = A_mem0.shape[1]
    d_ff = B_w_gate.shape[1]
    seg = A_seg_len if isinstance(A_seg_len, int) else min(32, s_len)
    rows = 2 * (n_mem + seg)
    n_g = n_heads // _HG

    def stage_view(w):
        return w.reshape(d_model // 16, 16 * n_heads, e)

    n_chunks = d_ff // (2 * _T)
    half = d_model // 2
    any_spec = pl.BlockSpec(memory_space=pl.ANY)
    out = pl.pallas_call(
        functools.partial(_kernel, n_heads=n_heads, n_mem=n_mem, seg=seg),
        out_shape=jax.ShapeDtypeStruct((s_len, d_model), _BF16),
        in_specs=[any_spec, pl.BlockSpec(memory_space=pltpu.VMEM)] + [any_spec] * 7,
        out_specs=any_spec,
        scratch_shapes=[
            pltpu.VMEM((n_g, d_model, 3 * _HG * e), _BF16),
            pltpu.VMEM((n_heads * e, d_model), _BF16),
            pltpu.VMEM((7, n_chunks, half, 2 * _T), _BF16),
            pltpu.VMEM((7, n_chunks * _T, half), _BF16),
            pltpu.VMEM((s_len + seg, d_model), _BF16),
            pltpu.VMEM((rows, d_model), _BF16),
            pltpu.VMEM((rows, d_model), _F32),
            pltpu.VMEM((2, 7, 2 * seg, half), _BF16),
            pltpu.VMEM((2, 7, 2 * seg, half), _F32),
            pltpu.VMEM((rows, rows), _F32),
            pltpu.VMEM((2, rows - seg, rows - seg), _F32),
            pltpu.SemaphoreType.DMA((3 * (d_model // _DCH),)),
            pltpu.SemaphoreType.DMA((2,)),
            pltpu.SemaphoreType.DMA((n_g,)),
            pltpu.SemaphoreType.DMA((3, n_chunks)),
            pltpu.SemaphoreType.DMA((s_len // seg // _OUT_CH,)),
        ],
        compiler_params=pltpu.CompilerParams(vmem_limit_bytes=110 * 1024 * 1024),
    )(
        A_x.reshape(s_len, d_model).astype(_BF16),
        A_mem0.reshape(n_mem, d_model).astype(_F32),
        stage_view(A_Wq).astype(_BF16), stage_view(A_Wk).astype(_BF16),
        stage_view(A_Wv).astype(_BF16),
        A_Wo.reshape(n_heads * e, d_model).astype(_BF16),
        B_w_gate.astype(_BF16), B_w_up.astype(_BF16), B_w_down.astype(_BF16),
    )
    return out.reshape(1, s_len, d_model).astype(A_x.dtype)
```

```python
import functools
import math

import jax
import jax.numpy as jnp
from jax import lax
import jax.experimental.pallas as pl
import jax.experimental.pallas.tpu as pltpu

_BF16 = jnp.bfloat16
_F32 = jnp.float32

_HG = 4
_T = 128
_DCH = 128
_OUT_CH = 4
_LEAD = 4
_WINDOW = 3
_D_BATCH = 2


def _layernorm(x):
    m = jnp.mean(x, axis=-1, keepdims=True)
    c = x - m
    v = jnp.mean(c * c, axis=-1, keepdims=True)
    return c * lax.rsqrt(v + 1e-5)


def _gelu(x):
    k = math.sqrt(2.0 / math.pi)
    return x * (0.5 * (1.0 + jnp.tanh(k * (x + 0.044715 * (x * x * x)))))


def _dot(a, b):
    return jnp.dot(a, b, preferred_element_type=_F32)


def _pack(x):
    return pltpu.bitcast(x.astype(_BF16), jnp.uint32)


def _unpack(words):
    return pltpu.bitcast(words, _BF16)


def _half(rows):
    return pl.ds(rows[0] // 2, rows[1] // 2)


def _lhs_blocks(a11, a12, a21, a22):
    return (a11 + a22, a21 + a22, a11, a22, a11 + a12, a21 - a11, a12 - a22)


def _rhs_blocks(b11, b12, b21, b22):
    return (b11 + b22, b11, b12 - b22, b21 - b11, b22, b11 + b12, b21 + b22)


def _out_blocks(m1, m2, m3, m4, m5, m6, m7):
    return (m1 + m4 - m5 + m7, m3 + m5, m2 + m4, m1 - m2 + m3 + m6)


def _attn_order(n_g, fill=()):
    order = []
    done = 0
    for g in range(n_g + 1):
        if g < n_g:
            order.append(("QKV", g))
        if g >= 1:
            order.append(("S", g - 1))
        if g >= 2:
            order.append(("O", g - 2))
        upto = (len(fill) * (g + 1)) // (n_g + 1)
        order.extend(fill[done:upto])
        done = upto
        if g >= 1:
            order.append(("PV", g - 1))
    return order


def _glu_order(n_c):
    order = []
    start = 0
    for c in range(n_c):
        order.append(("GU", c))
        if c - start == _D_BATCH and c < n_c - 1:
            order.append(("D", (start, c)))
            start = c
    if n_c - start > 1:
        order.append(("D", (start, n_c - 1)))
    order.append(("D", (n_c - 1, n_c)))
    return order


def _full_order(n_g, n_c):
    glu = _glu_order(n_c)
    return ([glu[0], ("ZFIN", 0)] + _attn_order(n_g, glu[1:-2])
            + [glu[-2], ("O", n_g - 1), ("YFIN", 0), glu[-1]])


def _kernel(x_hbm, mem0_ref, wq_hbm, wk_hbm, wv_hbm, wo_hbm, wg_hbm, wu_hbm, wd_hbm,
            out_hbm,
            wqkv, wo, wgu, wd, res, ha, oacc, hb, macc, bias2, bias1,
            sem_stage, sem_x, sem_o, sem_f, sem_out, *, n_heads, n_mem, seg):
    s_len, d_model = x_hbm.shape
    d_ff = wg_hbm.shape[1]
    e = wo.shape[0] // n_heads
    n_seg = s_len // seg
    n_g = n_heads // _HG
    n_chunks = d_ff // (2 * _T)
    n_c = n_chunks // 2
    n_dch = d_model // _DCH
    half = d_model // 2
    m2 = 2 * n_mem
    scale = e ** -0.5
    spare = n_seg

    queue = []
    issued = [0]

    def issue_upto(n):
        while issued[0] < min(n, len(queue)):
            queue[issued[0]]().start()
            issued[0] += 1

    def arrive(i):
        issue_upto(i + 1)
        queue[i]().wait()
        issue_upto(i + 1 + _WINDOW)

    x_head = (_LEAD + 2) * seg

    def x_copy(i):
        rows = pl.ds(0, x_head) if i == 0 else pl.ds(x_head, s_len - x_head)
        return pltpu.make_async_copy(x_hbm.at[rows], res.at[rows], sem_x.at[i])

    def wo_copy(g):
        rows = pl.ds(g * _HG * e, _HG * e)
        return pltpu.make_async_copy(wo_hbm.at[rows], wo.at[rows], sem_o.at[g])

    def load_attention_weights(stage):
        blk = _DCH // 16

        def stage_copy(w, c):
            return pltpu.make_async_copy(
                (wq_hbm, wk_hbm, wv_hbm)[w].at[pl.ds(c * blk, blk)],
                stage.at[w, pl.ds(c * blk, blk)], sem_stage.at[w * n_dch + c])

        queue.append(functools.partial(x_copy, 0))
        queue.extend(functools.partial(stage_copy, w, c)
                     for w in range(3) for c in range(n_dch))
        queue.extend(functools.partial(wo_copy, g) for g in range(n_g))
        issue_upto(_WINDOW)

        def score_fill(n_rows, layer_of_token):
            r_id = lax.broadcasted_iota(jnp.int32, (n_rows, n_rows), 0)
            c_id = lax.broadcasted_iota(jnp.int32, (n_rows, n_rows), 1)

            def layer_of(i):
                return jnp.where(i < m2, i // n_mem, layer_of_token(i - m2))

            same = layer_of(r_id) == layer_of(c_id)
            keep = same & ((r_id < m2) | (r_id >= c_id))
            return jnp.where(keep, 1.0, jnp.where(same, -1e9, -jnp.inf)).astype(_F32)

        bias2[...] = score_fill(m2 + 2 * seg, lambda i: i // seg)
        for layer in range(2):
            bias1[layer] = score_fill(m2 + seg, lambda i, layer=layer: layer)
        res[pl.ds(spare * seg, seg), :] = jnp.zeros((seg, d_model), _BF16)
        arrive(0)
        mem0 = mem0_ref[...]
        ha[_half((0, m2)), :] = _pack(jnp.concatenate([mem0, mem0], axis=0))

        pairs = n_heads // 2
        for w in range(3):
            src = stage.at[w].bitcast(jnp.uint32)
            for c in range(n_dch):
                arrive(1 + w * n_dch + c)

                def relayout(i, carry, src=src, w=w):
                    d0 = pl.multiple_of(i * 8, 8)
                    for j in range(pairs):
                        a = src[i, pl.ds(j, 8, stride=2 * pairs), :]
                        b = src[i, pl.ds(pairs + j, 8, stride=2 * pairs), :]
                        lo = (a & jnp.uint32(0xFFFF)) | (b << 16)
                        hi = (a >> 16) | (b & jnp.uint32(0xFFFF0000))
                        for h, val in ((2 * j, lo), (2 * j + 1, hi)):
                            col = (w * _HG + h % _HG) * e
                            wqkv[h // _HG, pl.ds(d0, 8), pl.ds(col, e)] = val
                    return carry

                lax.fori_loop(c * blk, (c + 1) * blk, relayout, 0)

    pl.run_scoped(load_attention_weights,
                  pltpu.VMEM((3, d_model // 16, 16 * n_heads, e), _BF16))
    wo_at = 1 + 3 * n_dch

    def rows_of(s):
        if isinstance(s, int):
            return pl.ds(s * seg, seg)
        return pl.ds(pl.multiple_of(s * seg, seg), seg)

    def load_segs(segs):
        return jnp.concatenate([res[rows_of(s), :] for s in segs], axis=0).astype(_F32)

    def prep_attn(vals):
        ha[_half((m2, vals.shape[0])), :] = _pack(_layernorm(vals))

    def prep_glu(buf, part, vals):
        h = _layernorm(vals)
        blocks = _lhs_blocks(h[:seg, :half], h[:seg, half:], h[seg:, :half], h[seg:, half:])
        for i, blk in enumerate(blocks):
            hb[buf, i, pl.ds(pl.multiple_of(part * (seg // 2), seg // 2), seg // 2), :] = _pack(blk)

    def finish_glu(buf, part, top, bottom):
        c11, c12, c21, c22 = _out_blocks(*(macc[buf, i, rows_of(part), :] for i in range(7)))
        z_top = (load_segs([top]) + jnp.concatenate([c11, c12], axis=1)).astype(_BF16)
        z_bot = (load_segs([bottom]) + jnp.concatenate([c21, c22], axis=1)).astype(_BF16)
        res[rows_of(top), :] = z_top
        res[rows_of(bottom), :] = z_bot
        return z_top

    def run(order, step=None, a_segs=(), layer=None, streaming=False):
        a_rows = m2 + len(a_segs) * seg
        if step is not None:
            part = step % 2
            buf = (step // 2) % 2
        qkv, probs, att, hid = {}, {}, {}, {}
        for op, i in order:
            if op == "ZFIN":
                done = jnp.where(step >= _LEAD, step - _LEAD, spare)
                z1 = finish_glu(1 - buf, part, step, done)
                prep_attn(jnp.concatenate(
                    [load_segs(a_segs[:1]), z1.astype(_F32)], axis=0))
            elif op == "QKV":
                qkv[i] = _dot(_unpack(ha[_half((0, a_rows)), :]), _unpack(wqkv[i])).astype(_BF16)
            elif op == "S":
                fill = bias2[...] if layer is None else bias1[layer]
                keep = fill > 0
                ps = []
                for h in range(_HG):
                    q = qkv[i][:, h * e:(h + 1) * e]
                    k = qkv[i][:, (_HG + h) * e:(_HG + h + 1) * e]
                    s = lax.dot_general(q, k, (((1,), (1,)), ((), ())),
                                        preferred_element_type=_F32)
                    s = jnp.where(keep, s * scale, fill)
                    p = jnp.exp(s - jnp.max(s, axis=-1, keepdims=True))
                    p = p / jnp.sum(p, axis=-1, keepdims=True)
                    ps.append(p.astype(_BF16))
                probs[i] = ps
            elif op == "PV":
                heads = []
                for h in range(_HG):
                    v = qkv[i][:, (2 * _HG + h) * e:(2 * _HG + h + 1) * e]
                    heads.append(_dot(probs[i][h], v).astype(_BF16))
                att[i] = jnp.concatenate(heads, axis=1)
            elif op == "O":
                if streaming:
                    arrive(wo_at + i)
                out = _dot(att[i], wo[pl.ds(i * _HG * e, _HG * e), :])
                if i == 0:
                    oacc[pl.ds(0, m2), :] = out[:m2]
                    oacc[pl.ds(m2, a_rows - m2), :] = load_segs(a_segs) + out[m2:]
                else:
                    oacc[pl.ds(0, a_rows), :] += out
            elif op == "YFIN":
                y = oacc[pl.ds(m2, a_rows - m2), :].astype(_BF16)
                for k, s in enumerate(a_segs):
                    res[rows_of(s), :] = y[k * seg:(k + 1) * seg]
                mem = oacc[pl.ds(0, m2), :]
                if layer is None:
                    prep_glu(1 - buf, part, y.astype(_F32))
                else:
                    row = lax.broadcasted_iota(jnp.int32, mem.shape, 0)
                    mine = (row >= layer * n_mem) & (row < (layer + 1) * n_mem)
                    mem = jnp.where(mine, mem, _unpack(ha[_half((0, m2)), :]).astype(_F32))
                ha[_half((0, m2)), :] = _pack(mem)
            elif op == "GU":
                c = part * n_c + i
                c11, c12, c21, c22 = _out_blocks(
                    *(_dot(_unpack(hb[buf, k]), _unpack(wgu[k, c])) for k in range(7)))
                hid[i] = [blk.astype(_BF16) for blk in _lhs_blocks(
                    *(_gelu(blk[:, :_T]) * blk[:, _T:] for blk in (c11, c12, c21, c22)))]
            elif op == "D":
                lo, hi = i
                rows = pl.ds(pl.multiple_of((part * n_c + lo) * (_T // 2), _T // 2),
                             (hi - lo) * (_T // 2))
                for k in range(7):
                    lhs = jnp.concatenate([hid[c][k] for c in range(lo, hi)], axis=1)
                    out = _dot(lhs, _unpack(wd[k, rows, :]))
                    if lo == 0:
                        macc[buf, k] = jnp.where(part == 0, out, macc[buf, k] + out)
                    else:
                        macc[buf, k] += out

    def loop(lo, hi, fn):
        def body(i, carry):
            fn(i)
            return carry
        lax.fori_loop(lo, hi, body, 0)

    attn_all = _attn_order(n_g) + [("O", n_g - 1), ("YFIN", 0)]

    def attn_one(layer, s, streaming=False):
        prep_attn(load_segs([s]))
        run(attn_all, a_segs=[s], layer=layer, streaming=streaming)

    def glu_four(buf, first):
        loop(0, 2, lambda part: prep_glu(
            buf, part, load_segs([first + 2 + part, first + part])))
        loop(2 * buf, 2 * buf + 2, lambda step: run(_glu_order(n_c), step=step))

    def head_start(raw_g, raw_u, raw_d):
        def raw_copy(w, c):
            start = c * 2 * _T
            cols = pl.ds(start if isinstance(c, int) else pl.multiple_of(start, 2 * _T), 2 * _T)
            src, dst = ((wg_hbm.at[:, cols], raw_g.at[c]), (wu_hbm.at[:, cols], raw_u.at[c]),
                        (wd_hbm.at[cols], raw_d.at[c]))[w]
            return pltpu.make_async_copy(src, dst, sem_f.at[w, c])

        def split(raw, c, r, dr, k, dk, store):
            quads = [raw[c, pl.ds(r + i * dr, 16), pl.ds(k + j * dk, _T)]
                     for i in range(2) for j in range(2)]
            blocks = list(_rhs_blocks(*(q.astype(_F32) for q in quads)))
            blocks[1], blocks[4] = quads[0], quads[3]
            for i, blk in enumerate(blocks):
                store(i, _pack(blk))

        def split_weights(c):
            for w in range(3):
                raw_copy(w, c).wait()
            for w, raw in enumerate((raw_g, raw_u)):
                for r in range(0, half, 16):
                    def store(i, val, r=r, w=w):
                        wgu[i, c, _half((r, 16)), pl.ds(w * _T, _T)] = val
                    split(raw, c, r, half, 0, _T, store)
            for r in range(0, _T, 16):
                for k in range(0, half, _T):
                    def store(i, val, r=r, k=k):
                        row = pl.multiple_of(c * (_T // 2) + r // 2, 8)
                        wd[i, pl.ds(row, 8), pl.ds(k, _T)] = val
                    split(raw_d, c, r, _T, k, half, store)

        attn_one(0, 0, streaming=True)
        for c in range(n_chunks):
            for w in range(3):
                raw_copy(w, c).start()
        loop(1, _LEAD, lambda s: attn_one(0, s))
        x_copy(1).start()
        loop(0, n_chunks, split_weights)

    pl.run_scoped(head_start,
                  pltpu.VMEM((n_chunks, d_model, 2 * _T), _BF16),
                  pltpu.VMEM((n_chunks, d_model, 2 * _T), _BF16),
                  pltpu.VMEM((n_chunks, 2 * _T, d_model), _BF16))

    macc[...] = jnp.zeros(macc.shape, _F32)
    glu_four(0, 0)
    loop(0, 2, lambda part: finish_glu(0, part, spare, part))
    x_copy(1).wait()

    def attn_step(j):
        segs = [j + _LEAD, j]
        prep_attn(load_segs(segs))
        run(attn_all, step=j, a_segs=segs)

    loop(0, 2, attn_step)

    def out_copy(c):
        n = _OUT_CH * seg
        return pltpu.make_async_copy(
            res.at[pl.ds(c * n, n)], out_hbm.at[pl.ds(c * n, n)], sem_out.at[c])

    n_out = n_seg // _OUT_CH
    n_main = n_seg - _LEAD
    full = _full_order(n_g, n_c)

    def full_step(j):
        run(full, step=j, a_segs=[j + _LEAD, j])
        final = j + 1 - _LEAD

        @pl.when((final > 0) & (final % _OUT_CH == 0))
        def _():
            out_copy(final // _OUT_CH - 1).start()

    loop(2, n_main, full_step)

    buf = (n_main // 2) % 2
    loop(0, 2, lambda part: finish_glu(
        1 - buf, part, n_main + part, n_main - _LEAD + part))
    loop(2 * buf, 2 * buf + 2, lambda step: run(_glu_order(n_c), step=step))
    loop(0, 2, lambda part: finish_glu(
        buf, part, n_main + 2 + part, n_main - 2 + part))
    out_copy(n_out - 2).start()
    loop(n_main, n_seg, lambda s: attn_one(1, s))
    glu_four(0, n_main)
    loop(0, 2, lambda part: finish_glu(0, part, n_main + 2 + part, n_main + part))
    out_copy(n_out - 1).start()
    for c in range(n_out):
        out_copy(c).wait()


@jax.jit
def pallas_interleave_layers__memory_aug_recurrent_mem_tr__glu_gated_geglu__prompt_kernel(
    A_x: jax.Array,
    A_mem0: jax.Array,
    A_Wq: jax.Array,
    A_Wk: jax.Array,
    A_Wv: jax.Array,
    A_Wo: jax.Array,
    A_seg_len: jax.Array,
    B_x: jax.Array,
    B_w_gate: jax.Array,
    B_w_up: jax.Array,
    B_w_down: jax.Array,
):
    del B_x
    _, s_len, d_model = A_x.shape
    _, n_heads, e = A_Wq.shape
    n_mem = A_mem0.shape[1]
    d_ff = B_w_gate.shape[1]
    seg = A_seg_len if isinstance(A_seg_len, int) else min(32, s_len)
    rows = 2 * (n_mem + seg)
    n_g = n_heads // _HG

    def stage_view(w):
        return w.reshape(d_model // 16, 16 * n_heads, e)

    n_chunks = d_ff // (2 * _T)
    half = d_model // 2
    any_spec = pl.BlockSpec(memory_space=pl.ANY)
    out = pl.pallas_call(
        functools.partial(_kernel, n_heads=n_heads, n_mem=n_mem, seg=seg),
        out_shape=jax.ShapeDtypeStruct((s_len, d_model), _BF16),
        in_specs=[any_spec, pl.BlockSpec(memory_space=pltpu.VMEM)] + [any_spec] * 7,
        out_specs=any_spec,
        scratch_shapes=[
            pltpu.VMEM((n_g, half, 3 * _HG * e), jnp.uint32),
            pltpu.VMEM((n_heads * e, d_model), _BF16),
            pltpu.VMEM((7, n_chunks, half // 2, 2 * _T), jnp.uint32),
            pltpu.VMEM((7, n_chunks * _T // 2, half), jnp.uint32),
            pltpu.VMEM((s_len + seg, d_model), _BF16),
            pltpu.VMEM((rows // 2, d_model), jnp.uint32),
            pltpu.VMEM((rows, d_model), _F32),
            pltpu.VMEM((2, 7, seg, half), jnp.uint32),
            pltpu.VMEM((2, 7, 2 * seg, half), _F32),
            pltpu.VMEM((rows, rows), _F32),
            pltpu.VMEM((2, rows - seg, rows - seg), _F32),
            pltpu.SemaphoreType.DMA((3 * (d_model // _DCH),)),
            pltpu.SemaphoreType.DMA((2,)),
            pltpu.SemaphoreType.DMA((n_g,)),
            pltpu.SemaphoreType.DMA((3, n_chunks)),
            pltpu.SemaphoreType.DMA((s_len // seg // _OUT_CH,)),
        ],
        compiler_params=pltpu.CompilerParams(vmem_limit_bytes=110 * 1024 * 1024),
    )(
        A_x.reshape(s_len, d_model).astype(_BF16),
        A_mem0.reshape(n_mem, d_model).astype(_F32),
        stage_view(A_Wq).astype(_BF16), stage_view(A_Wk).astype(_BF16),
        stage_view(A_Wv).astype(_BF16),
        A_Wo.reshape(n_heads * e, d_model).astype(_BF16),
        B_w_gate.astype(_BF16), B_w_up.astype(_BF16), B_w_down.astype(_BF16),
    )
    return out.reshape(1, s_len, d_model).astype(A_x.dtype)
```

```python
import functools
import math

import jax
import jax.numpy as jnp
from jax import lax
import jax.experimental.pallas as pl
import jax.experimental.pallas.tpu as pltpu

_BF16 = jnp.bfloat16
_F32 = jnp.float32

_HG = 4
_T = 128
_DCH = 128
_OUT_CH = 4
_LEAD = 4
_WINDOW = 4
_D_BATCH = 3
_FIRST_GLU_AT = 4


def _layernorm(x):
    m = jnp.mean(x, axis=-1, keepdims=True)
    c = x - m
    v = jnp.mean(c * c, axis=-1, keepdims=True)
    return c * lax.rsqrt(v + 1e-5)


def _gelu(x):
    k = math.sqrt(2.0 / math.pi)
    return x * (0.5 * (1.0 + jnp.tanh(k * (x + 0.044715 * (x * x * x)))))


def _dot(a, b):
    return jnp.dot(a, b, preferred_element_type=_F32)


def _pack(x):
    return pltpu.bitcast(x.astype(_BF16), jnp.uint32)


def _unpack(words):
    return pltpu.bitcast(words, _BF16)


def _half(rows):
    return pl.ds(rows[0] // 2, rows[1] // 2)


def _lhs_blocks(a11, a12, a21, a22):
    return (a11 + a22, a21 + a22, a11, a22, a11 + a12, a21 - a11, a12 - a22)


def _rhs_blocks(b11, b12, b21, b22):
    return (b11 + b22, b11, b12 - b22, b21 - b11, b22, b11 + b12, b21 + b22)


def _out_blocks(m1, m2, m3, m4, m5, m6, m7):
    return (m1 + m4 - m5 + m7, m3 + m5, m2 + m4, m1 - m2 + m3 + m6)


def _attn_order(n_g, fill=()):
    order = []
    done = 0
    for g in range(n_g + 1):
        if g < n_g:
            order.append(("QKV", g))
        if g >= 1:
            order.append(("S", g - 1))
        if g >= 2:
            order.append(("O", g - 2))
        upto = (len(fill) * (g + 1)) // (n_g + 1)
        order.extend(fill[done:upto])
        done = upto
        if g >= 1:
            order.append(("PV", g - 1))
    return order


def _glu_order(n_c):
    order = []
    start = 0
    for c in range(n_c):
        order.append(("GU", c))
        if c - start == _D_BATCH and c < n_c - 1:
            order.append(("D", (start, c)))
            start = c
    if n_c - start > 1:
        order.append(("D", (start, n_c - 1)))
    order.append(("D", (n_c - 1, n_c)))
    return order


def _full_order(n_g, n_c):
    glu = _glu_order(n_c)
    return ([glu[0], ("ZFIN", 0)] + _attn_order(n_g, glu[1:-2])
            + [glu[-2], ("O", n_g - 1), ("YFIN", 0), glu[-1]])


def _kernel(x_hbm, mem0_ref, wq_hbm, wk_hbm, wv_hbm, wo_hbm, wg_hbm, wu_hbm, wd_hbm,
            out_hbm,
            wq, wk, wv, wo, wgu, wd, res, ha, h0, early, oacc, hb, macc, bias2, bias1,
            sem_stage, sem_x, sem_o, sem_f, sem_out, *, n_heads, n_mem, seg):
    s_len, d_model = x_hbm.shape
    d_ff = wg_hbm.shape[1]
    e = wo.shape[0] // n_heads
    n_seg = s_len // seg
    n_g = n_heads // _HG
    n_chunks = d_ff // (2 * _T)
    n_c = n_chunks // 2
    n_dch = d_model // _DCH
    half = d_model // 2
    m2 = 2 * n_mem
    scale = e ** -0.5
    spare = n_seg
    wqkv = (wq, wk, wv)

    x_head = (_LEAD + 2) * seg

    def x_copy(i):
        rows = pl.ds(0, x_head) if i == 0 else pl.ds(x_head, s_len - x_head)
        return pltpu.make_async_copy(x_hbm.at[rows], res.at[rows], sem_x.at[i])

    def wo_copy(g):
        rows = pl.ds(g * _HG * e, _HG * e)
        return pltpu.make_async_copy(wo_hbm.at[rows], wo.at[rows], sem_o.at[g])

    def rows_of(s):
        if isinstance(s, int):
            return pl.ds(s * seg, seg)
        return pl.ds(pl.multiple_of(s * seg, seg), seg)

    def load_segs(segs):
        return jnp.concatenate([res[rows_of(s), :] for s in segs], axis=0).astype(_F32)

    def loop(lo, hi, fn):
        def body(i, carry):
            fn(i)
            return carry
        lax.fori_loop(lo, hi, body, 0)

    def project_early(w, g):
        early[w, g] = _pack(_dot(_unpack(h0[...]), _unpack(wqkv[w][g])))

    def project(n_rows, g):
        h = _unpack(ha[_half((0, n_rows)), :])
        return [_dot(h, _unpack(w[g])).astype(_BF16) for w in wqkv]

    def load_attention_weights(stage):
        blk = _DCH // 16

        def stage_copy(w, c):
            start = c * blk if isinstance(c, int) else pl.multiple_of(c * blk, blk)
            return pltpu.make_async_copy(
                (wq_hbm, wk_hbm, wv_hbm)[w].at[pl.ds(start, blk)],
                stage.at[w, pl.ds(start, blk)], sem_stage.at[w, c])

        x_copy(0).start()
        for c in range(_WINDOW):
            stage_copy(0, c).start()

        def score_fill(n_rows, layer_of_token):
            r_id = lax.broadcasted_iota(jnp.int32, (n_rows, n_rows), 0)
            c_id = lax.broadcasted_iota(jnp.int32, (n_rows, n_rows), 1)

            def layer_of(i):
                return jnp.where(i < m2, i // n_mem, layer_of_token(i - m2))

            same = layer_of(r_id) == layer_of(c_id)
            keep = same & ((r_id < m2) | (r_id >= c_id))
            return jnp.where(keep, 1.0, jnp.where(same, -1e9, -jnp.inf)).astype(_F32)

        bias2[...] = score_fill(m2 + 2 * seg, lambda i: i // seg)
        for layer in range(2):
            bias1[layer] = score_fill(m2 + seg, lambda i, layer=layer: layer)
        res[pl.ds(spare * seg, seg), :] = jnp.zeros((seg, d_model), _BF16)
        x_copy(0).wait()
        mem0 = mem0_ref[...]
        mem0 = _pack(jnp.concatenate([mem0, mem0], axis=0))
        ha[_half((0, m2)), :] = mem0
        h0[_half((0, m2)), :] = mem0
        for k, s in enumerate((0, _LEAD, _LEAD + 1)):
            h0[_half((m2 + k * seg, seg)), :] = _pack(_layernorm(load_segs([s])))

        for w in range(3):
            src = stage.at[w].bitcast(jnp.uint32)

            def relayout(i, src=src, w=w):
                d0 = pl.multiple_of(i * 8, 8)
                for part in range(n_heads // 16):
                    v = [src[i, pl.ds(d * (n_heads // 2) + part * 8, 8), :] for d in range(16)]
                    even = jnp.stack([(v[2 * p] & jnp.uint32(0xFFFF)) | (v[2 * p + 1] << 16)
                                      for p in range(8)])
                    odd = jnp.stack([(v[2 * p] >> 16) | (v[2 * p + 1] & jnp.uint32(0xFFFF0000))
                                     for p in range(8)])
                    for k, val in enumerate((even, odd)):
                        val = jnp.swapaxes(val, 0, 1)
                        for j in range(8):
                            h = 2 * (part * 8 + j) + k
                            wqkv[w][h // _HG, pl.ds(d0, 8), pl.ds((h % _HG) * e, e)] = val[j]

            def chunk(c, w=w, relayout=relayout):
                stage_copy(w, c).wait()

                @pl.when(c + _WINDOW < n_dch)
                def _():
                    stage_copy(w, c + _WINDOW).start()

                @pl.when(c + _WINDOW >= n_dch)
                def _():
                    nxt = c + _WINDOW - n_dch
                    (stage_copy(w + 1, nxt) if w < 2 else wo_copy(nxt)).start()

                loop(c * blk, (c + 1) * blk, relayout)
                if w > 0:
                    project_early(w - 1, c)

            loop(0, n_dch, chunk)

    pl.run_scoped(load_attention_weights,
                  pltpu.VMEM((3, d_model // 16, 16 * n_heads, e), _BF16))

    def prep_attn(vals):
        ha[_half((m2, vals.shape[0])), :] = _pack(_layernorm(vals))

    def prep_glu(buf, part, vals):
        h = _layernorm(vals)
        blocks = _lhs_blocks(h[:seg, :half], h[:seg, half:], h[seg:, :half], h[seg:, half:])
        for i, blk in enumerate(blocks):
            hb[buf, i, pl.ds(pl.multiple_of(part * (seg // 2), seg // 2), seg // 2), :] = _pack(blk)

    def finish_glu(buf, part, top, bottom):
        c11, c12, c21, c22 = _out_blocks(*(macc[buf, i, rows_of(part), :] for i in range(7)))
        z_top = (load_segs([top]) + jnp.concatenate([c11, c12], axis=1)).astype(_BF16)
        z_bot = (load_segs([bottom]) + jnp.concatenate([c21, c22], axis=1)).astype(_BF16)
        res[rows_of(top), :] = z_top
        res[rows_of(bottom), :] = z_bot
        return z_top

    def run(order, step=None, a_segs=(), layer=None, first=False, side=None):
        a_rows = m2 + len(a_segs) * seg
        if step is not None:
            part = step % 2
            buf = (step // 2) % 2
        qkv, probs, att, hid = {}, {}, {}, {}
        for op, i in order:
            if op == "ZFIN":
                done = jnp.where(step >= _LEAD, step - _LEAD, spare)
                z1 = finish_glu(1 - buf, part, step, done)
                prep_attn(jnp.concatenate(
                    [load_segs(a_segs[:1]), z1.astype(_F32)], axis=0))
            elif op == "SIDE":
                side(i)
            elif op == "QKV" and first and layer is not None:
                project_early(2, i)
                qkv[i] = [_unpack(early[w, i, _half((0, a_rows)), :]) for w in range(3)]
            elif op == "QKV" and first:
                rows = pl.ds(pl.multiple_of((m2 + (1 + step) * seg) // 2, 8), seg // 2)
                qkv[i] = [
                    jnp.concatenate([t[:m2], _unpack(early[w, i, rows, :]), t[m2:]], axis=0)
                    for w, t in enumerate(project(m2 + seg, i))]
            elif op == "QKV":
                qkv[i] = project(a_rows, i)
            elif op == "S":
                fill = bias2[...] if layer is None else bias1[layer]
                keep = fill > 0
                ps = []
                for h in range(_HG):
                    q = qkv[i][0][:, h * e:(h + 1) * e]
                    k = qkv[i][1][:, h * e:(h + 1) * e]
                    s = lax.dot_general(q, k, (((1,), (1,)), ((), ())),
                                        preferred_element_type=_F32)
                    s = jnp.where(keep, s * scale, fill)
                    p = jnp.exp(s - jnp.max(s, axis=-1, keepdims=True))
                    p = p / jnp.sum(p, axis=-1, keepdims=True)
                    ps.append(p.astype(_BF16))
                probs[i] = ps
            elif op == "PV":
                heads = []
                for h in range(_HG):
                    v = qkv[i][2][:, h * e:(h + 1) * e]
                    heads.append(_dot(probs[i][h], v).astype(_BF16))
                att[i] = jnp.concatenate(heads, axis=1)
            elif op == "O":
                if first and layer is not None:
                    wo_copy(i).wait()
                out = _dot(att[i], wo[pl.ds(i * _HG * e, _HG * e), :])
                if i == 0:
                    oacc[pl.ds(0, m2), :] = out[:m2]
                    oacc[pl.ds(m2, a_rows - m2), :] = load_segs(a_segs) + out[m2:]
                else:
                    oacc[pl.ds(0, a_rows), :] += out
            elif op == "YFIN":
                y = oacc[pl.ds(m2, a_rows - m2), :].astype(_BF16)
                for k, s in enumerate(a_segs):
                    res[rows_of(s), :] = y[k * seg:(k + 1) * seg]
                mem = oacc[pl.ds(0, m2), :]
                if layer is None:
                    prep_glu(1 - buf, part, y.astype(_F32))
                else:
                    row = lax.broadcasted_iota(jnp.int32, mem.shape, 0)
                    mine = (row >= layer * n_mem) & (row < (layer + 1) * n_mem)
                    mem = jnp.where(mine, mem, _unpack(ha[_half((0, m2)), :]).astype(_F32))
                ha[_half((0, m2)), :] = _pack(mem)
            elif op == "GU":
                c = part * n_c + i
                c11, c12, c21, c22 = _out_blocks(
                    *(_dot(_unpack(hb[buf, k]), _unpack(wgu[k, c])) for k in range(7)))
                hid[i] = [blk.astype(_BF16) for blk in _lhs_blocks(
                    *(_gelu(blk[:, :_T]) * blk[:, _T:] for blk in (c11, c12, c21, c22)))]
            elif op == "D":
                lo, hi = i
                rows = pl.ds(pl.multiple_of((part * n_c + lo) * (_T // 2), _T // 2),
                             (hi - lo) * (_T // 2))
                for k in range(7):
                    lhs = jnp.concatenate([hid[c][k] for c in range(lo, hi)], axis=1)
                    out = _dot(lhs, _unpack(wd[k, rows, :]))
                    if lo == 0:
                        macc[buf, k] = jnp.where(part == 0, out, macc[buf, k] + out)
                    else:
                        macc[buf, k] += out

    attn_all = _attn_order(n_g) + [("O", n_g - 1), ("YFIN", 0)]

    def attn_one(layer, s):
        prep_attn(load_segs([s]))
        run(attn_all, a_segs=[s], layer=layer)

    def glu_four(buf, first):
        loop(0, 2, lambda part: prep_glu(
            buf, part, load_segs([first + 2 + part, first + part])))
        loop(2 * buf, 2 * buf + 2, lambda step: run(_glu_order(n_c), step=step))

    def head_start(raw_g, raw_u, raw_d):
        def raw_copy(w, c):
            start = c * 2 * _T
            cols = pl.ds(start if isinstance(c, int) else pl.multiple_of(start, 2 * _T), 2 * _T)
            src, dst = ((wg_hbm.at[:, cols], raw_g.at[c]), (wu_hbm.at[:, cols], raw_u.at[c]),
                        (wd_hbm.at[cols], raw_d.at[c]))[w]
            return pltpu.make_async_copy(src, dst, sem_f.at[w, c])

        def split(raw, c, r, dr, k, dk, store):
            quads = [pltpu.bitcast(raw[c, pl.ds(r + i * dr, 16), pl.ds(k + j * dk, _T)],
                                   jnp.uint32)
                     for i in range(2) for j in range(2)]
            even = _rhs_blocks(*(pltpu.bitcast(q << 16, _F32) for q in quads))
            odd = _rhs_blocks(
                *(pltpu.bitcast(q & jnp.uint32(0xFFFF0000), _F32) for q in quads))
            for i, pair in enumerate(zip(even, odd)):
                if i in (1, 4):
                    store(i, quads[0 if i == 1 else 3])
                else:
                    packed = pltpu.pack_elementwise(list(pair), packed_dtype=_BF16)
                    store(i, pltpu.bitcast(packed, jnp.uint32))

        def split_piece(c, n):
            w, n = divmod(n, half // 16)
            if w < 2:
                def store(i, val):
                    wgu[i, c, _half((n * 16, 16)), pl.ds(w * _T, _T)] = val
                split((raw_g, raw_u)[w], c, n * 16, half, 0, _T, store)
            else:
                r, k = divmod(n, half // _T)

                def store(i, val):
                    row = pl.multiple_of(c * (_T // 2) + r * 8, 8)
                    wd[i, pl.ds(row, 8), pl.ds(k * _T, _T)] = val
                split(raw_d, c, r * 16, _T, k * _T, half, store)

        def fetch(_):
            for c in range(n_chunks):
                for w in range(3):
                    raw_copy(w, c).start()

        def split_chunk(c):
            for w in range(3):
                raw_copy(w, c).wait()
            for n in range(3 * (half // 16)):
                split_piece(c, n)

        for g in range(_WINDOW, n_g):
            wo_copy(g).start()
        order = list(attn_all)
        order.insert(order.index(("O", _FIRST_GLU_AT)) + 1, ("SIDE", 0))
        run(order, a_segs=[0], layer=0, first=True, side=fetch)
        loop(1, _LEAD, lambda s: attn_one(0, s))
        x_copy(1).start()
        loop(0, n_chunks, split_chunk)

    pl.run_scoped(head_start,
                  pltpu.VMEM((n_chunks, d_model, 2 * _T), _BF16),
                  pltpu.VMEM((n_chunks, d_model, 2 * _T), _BF16),
                  pltpu.VMEM((n_chunks, 2 * _T, d_model), _BF16))

    macc[...] = jnp.zeros(macc.shape, _F32)
    glu_four(0, 0)
    loop(0, 2, lambda part: finish_glu(0, part, spare, part))
    x_copy(1).wait()

    def attn_step(j):
        prep_attn(load_segs([j]))
        run(attn_all, step=j, a_segs=[j + _LEAD, j], first=True)

    loop(0, 2, attn_step)

    def out_copy(c):
        n = _OUT_CH * seg
        return pltpu.make_async_copy(
            res.at[pl.ds(c * n, n)], out_hbm.at[pl.ds(c * n, n)], sem_out.at[c])

    n_out = n_seg // _OUT_CH
    n_main = n_seg - _LEAD
    full = _full_order(n_g, n_c)

    def full_step(j):
        run(full, step=j, a_segs=[j + _LEAD, j])
        final = j + 1 - _LEAD

        @pl.when((final > 0) & (final % _OUT_CH == 0))
        def _():
            out_copy(final // _OUT_CH - 1).start()

    loop(2, n_main, full_step)

    buf = (n_main // 2) % 2
    loop(0, 2, lambda part: finish_glu(
        1 - buf, part, n_main + part, n_main - _LEAD + part))
    loop(2 * buf, 2 * buf + 2, lambda step: run(_glu_order(n_c), step=step))
    loop(0, 2, lambda part: finish_glu(
        buf, part, n_main + 2 + part, n_main - 2 + part))
    out_copy(n_out - 2).start()
    loop(n_main, n_seg, lambda s: attn_one(1, s))
    glu_four(0, n_main)
    loop(0, 2, lambda part: finish_glu(0, part, n_main + 2 + part, n_main + part))
    out_copy(n_out - 1).start()
    for c in range(n_out):
        out_copy(c).wait()


@jax.jit
def pallas_interleave_layers__memory_aug_recurrent_mem_tr__glu_gated_geglu__prompt_kernel(
    A_x: jax.Array,
    A_mem0: jax.Array,
    A_Wq: jax.Array,
    A_Wk: jax.Array,
    A_Wv: jax.Array,
    A_Wo: jax.Array,
    A_seg_len: jax.Array,
    B_x: jax.Array,
    B_w_gate: jax.Array,
    B_w_up: jax.Array,
    B_w_down: jax.Array,
):
    del B_x
    _, s_len, d_model = A_x.shape
    _, n_heads, e = A_Wq.shape
    n_mem = A_mem0.shape[1]
    d_ff = B_w_gate.shape[1]
    seg = A_seg_len if isinstance(A_seg_len, int) else min(32, s_len)
    rows = 2 * (n_mem + seg)
    rows_early = 2 * n_mem + 3 * seg
    n_g = n_heads // _HG

    def stage_view(w):
        return w.reshape(d_model // 16, 16 * n_heads, e)

    n_chunks = d_ff // (2 * _T)
    half = d_model // 2
    any_spec = pl.BlockSpec(memory_space=pl.ANY)
    out = pl.pallas_call(
        functools.partial(_kernel, n_heads=n_heads, n_mem=n_mem, seg=seg),
        out_shape=jax.ShapeDtypeStruct((s_len, d_model), _BF16),
        in_specs=[any_spec, pl.BlockSpec(memory_space=pltpu.VMEM)] + [any_spec] * 7,
        out_specs=any_spec,
        scratch_shapes=[
            pltpu.VMEM((n_g, half, _HG * e), jnp.uint32),
            pltpu.VMEM((n_g, half, _HG * e), jnp.uint32),
            pltpu.VMEM((n_g, half, _HG * e), jnp.uint32),
            pltpu.VMEM((n_heads * e, d_model), _BF16),
            pltpu.VMEM((7, n_chunks, half // 2, 2 * _T), jnp.uint32),
            pltpu.VMEM((7, n_chunks * _T // 2, half), jnp.uint32),
            pltpu.VMEM((s_len + seg, d_model), _BF16),
            pltpu.VMEM((rows // 2, d_model), jnp.uint32),
            pltpu.VMEM((rows_early // 2, d_model), jnp.uint32),
            pltpu.VMEM((3, n_g, rows_early // 2, _HG * e), jnp.uint32),
            pltpu.VMEM((rows, d_model), _F32),
            pltpu.VMEM((2, 7, seg, half), jnp.uint32),
            pltpu.VMEM((2, 7, 2 * seg, half), _F32),
            pltpu.VMEM((rows, rows), _F32),
            pltpu.VMEM((2, rows - seg, rows - seg), _F32),
            pltpu.SemaphoreType.DMA((3, d_model // _DCH)),
            pltpu.SemaphoreType.DMA((2,)),
            pltpu.SemaphoreType.DMA((n_g,)),
            pltpu.SemaphoreType.DMA((3, n_chunks)),
            pltpu.SemaphoreType.DMA((s_len // seg // _OUT_CH,)),
        ],
        compiler_params=pltpu.CompilerParams(vmem_limit_bytes=110 * 1024 * 1024),
    )(
        A_x.reshape(s_len, d_model).astype(_BF16),
        A_mem0.reshape(n_mem, d_model).astype(_F32),
        stage_view(A_Wq).astype(_BF16), stage_view(A_Wk).astype(_BF16),
        stage_view(A_Wv).astype(_BF16),
        A_Wo.reshape(n_heads * e, d_model).astype(_BF16),
        B_w_gate.astype(_BF16), B_w_up.astype(_BF16), B_w_down.astype(_BF16),
    )
    return out.reshape(1, s_len, d_model).astype(A_x.dtype)
```

```python
import functools
import math

import jax
import jax.numpy as jnp
from jax import lax
import jax.experimental.pallas as pl
import jax.experimental.pallas.tpu as pltpu

_BF16 = jnp.bfloat16
_F32 = jnp.float32

_HG = 4
_T = 128
_DCH = 128
_OUT_CH = 4
_LEAD = 4
_WINDOW = 4
_D_BATCH = 3
_FIRST_GLU_AT = 4


def _layernorm(x):
    m = jnp.mean(x, axis=-1, keepdims=True)
    c = x - m
    v = jnp.mean(c * c, axis=-1, keepdims=True)
    return c * lax.rsqrt(v + 1e-5)


def _gelu(x):
    k = math.sqrt(2.0 / math.pi)
    return x * (0.5 * (1.0 + jnp.tanh(k * (x + 0.044715 * (x * x * x)))))


def _dot(a, b):
    return jnp.dot(a, b, preferred_element_type=_F32)


def _pack(x):
    return pltpu.bitcast(x.astype(_BF16), jnp.uint32)


def _unpack(words):
    return pltpu.bitcast(words, _BF16)


def _half(rows):
    return pl.ds(rows[0] // 2, rows[1] // 2)


def _lhs_blocks(a11, a12, a21, a22):
    return (a11 + a22, a21 + a22, a11, a22, a11 + a12, a21 - a11, a12 - a22)


def _rhs_blocks(b11, b12, b21, b22):
    return (b11 + b22, b11, b12 - b22, b21 - b11, b22, b11 + b12, b21 + b22)


def _out_blocks(m1, m2, m3, m4, m5, m6, m7):
    return (m1 + m4 - m5 + m7, m3 + m5, m2 + m4, m1 - m2 + m3 + m6)


def _attn_order(n_g, fill=()):
    order = []
    done = 0
    for g in range(n_g + 1):
        if g >= 1:
            order.append(("S", g - 1))
        if g >= 2:
            order.append(("O", g - 2))
        upto = (len(fill) * (g + 1)) // (n_g + 1)
        order.extend(fill[done:upto])
        done = upto
        if g < n_g:
            order.append(("QKV", g))
        if g >= 1:
            order.append(("PV", g - 1))
    return order


def _glu_order(n_c):
    order = []
    start = 0
    for c in range(n_c):
        order.append(("GU", c))
        if c - start == _D_BATCH and c < n_c - 1:
            order.append(("D", (start, c)))
            start = c
    if n_c - start > 1:
        order.append(("D", (start, n_c - 1)))
    order.append(("D", (n_c - 1, n_c)))
    return order


def _full_order(n_g, n_c):
    glu = _glu_order(n_c)
    return ([glu[0], ("ZFIN", 0)] + _attn_order(n_g, glu[1:-2])
            + [glu[-2], ("O", n_g - 1), ("YFIN", 0), glu[-1]])


def _kernel(x_hbm, mem0_ref, wq_hbm, wk_hbm, wv_hbm, wo_hbm, wg_hbm, wu_hbm, wd_hbm,
            out_hbm,
            wq, wk, wv, wo, wgu, wd, res, ha, h0, early, oacc, hb, macc, bias2, bias1,
            sem_stage, sem_x, sem_o, sem_f, sem_out, *, n_heads, n_mem, seg):
    s_len, d_model = x_hbm.shape
    d_ff = wg_hbm.shape[1]
    e = wo.shape[0] // n_heads
    n_seg = s_len // seg
    n_g = n_heads // _HG
    n_chunks = d_ff // (2 * _T)
    n_c = n_chunks // 2
    n_dch = d_model // _DCH
    half = d_model // 2
    m2 = 2 * n_mem
    scale = e ** -0.5
    spare = n_seg
    wqkv = (wq, wk, wv)

    x_head = (_LEAD + 2) * seg

    def x_copy(i):
        rows = pl.ds(0, x_head) if i == 0 else pl.ds(x_head, s_len - x_head)
        return pltpu.make_async_copy(x_hbm.at[rows], res.at[rows], sem_x.at[i])

    def wo_copy(g):
        rows = pl.ds(g * _HG * e, _HG * e)
        return pltpu.make_async_copy(wo_hbm.at[rows], wo.at[rows], sem_o.at[g])

    def rows_of(s):
        if isinstance(s, int):
            return pl.ds(s * seg, seg)
        return pl.ds(pl.multiple_of(s * seg, seg), seg)

    def load_segs(segs):
        return jnp.concatenate([res[rows_of(s), :] for s in segs], axis=0).astype(_F32)

    def loop(lo, hi, fn):
        def body(i, carry):
            fn(i)
            return carry
        lax.fori_loop(lo, hi, body, 0)

    def project_early(w, g):
        early[w, g] = _pack(_dot(_unpack(h0[...]), _unpack(wqkv[w][g])))

    def project(n_rows, g):
        h = _unpack(ha[_half((0, n_rows)), :])
        return [_dot(h, _unpack(w[g])).astype(_BF16) for w in wqkv]

    def load_attention_weights(stage):
        blk = _DCH // 16

        def stage_copy(w, c):
            start = c * blk if isinstance(c, int) else pl.multiple_of(c * blk, blk)
            return pltpu.make_async_copy(
                (wq_hbm, wk_hbm, wv_hbm)[w].at[pl.ds(start, blk)],
                stage.at[w, pl.ds(start, blk)], sem_stage.at[w, c])

        x_copy(0).start()
        for c in range(_WINDOW):
            stage_copy(0, c).start()

        def score_fill(n_rows, layer_of_token):
            r_id = lax.broadcasted_iota(jnp.int32, (n_rows, n_rows), 0)
            c_id = lax.broadcasted_iota(jnp.int32, (n_rows, n_rows), 1)

            def layer_of(i):
                return jnp.where(i < m2, i // n_mem, layer_of_token(i - m2))

            same = layer_of(r_id) == layer_of(c_id)
            keep = same & ((r_id < m2) | (r_id >= c_id))
            return jnp.where(keep, 1.0, jnp.where(same, -1e9, -jnp.inf)).astype(_F32)

        bias2[...] = score_fill(m2 + 2 * seg, lambda i: i // seg)
        for layer in range(2):
            bias1[layer] = score_fill(m2 + seg, lambda i, layer=layer: layer)
        res[pl.ds(spare * seg, seg), :] = jnp.zeros((seg, d_model), _BF16)
        x_copy(0).wait()
        mem0 = mem0_ref[...].astype(_F32)
        mem0 = _pack(jnp.concatenate([mem0, mem0], axis=0))
        ha[_half((0, m2)), :] = mem0
        h0[_half((0, m2)), :] = mem0
        for k, s in enumerate((0, _LEAD, _LEAD + 1)):
            h0[_half((m2 + k * seg, seg)), :] = _pack(_layernorm(load_segs([s])))

        for w in range(3):
            src = stage.at[w].bitcast(jnp.uint32)

            def relayout(i, src=src, w=w):
                d0 = pl.multiple_of(i * 8, 8)
                for part in range(n_heads // 16):
                    v = [src[i, pl.ds(d * (n_heads // 2) + part * 8, 8), :] for d in range(16)]
                    even = jnp.stack([(v[2 * p] & jnp.uint32(0xFFFF)) | (v[2 * p + 1] << 16)
                                      for p in range(8)])
                    odd = jnp.stack([(v[2 * p] >> 16) | (v[2 * p + 1] & jnp.uint32(0xFFFF0000))
                                     for p in range(8)])
                    for k, val in enumerate((even, odd)):
                        val = jnp.swapaxes(val, 0, 1)
                        for j in range(8):
                            h = 2 * (part * 8 + j) + k
                            wqkv[w][h // _HG, pl.ds(d0, 8), pl.ds((h % _HG) * e, e)] = val[j]

            def chunk(c, w=w, relayout=relayout):
                stage_copy(w, c).wait()

                @pl.when(c + _WINDOW < n_dch)
                def _():
                    stage_copy(w, c + _WINDOW).start()

                @pl.when(c + _WINDOW >= n_dch)
                def _():
                    nxt = c + _WINDOW - n_dch
                    (stage_copy(w + 1, nxt) if w < 2 else wo_copy(nxt)).start()

                loop(c * blk, (c + 1) * blk, relayout)
                if w > 0:
                    project_early(w - 1, c)

            loop(0, n_dch, chunk)

    pl.run_scoped(load_attention_weights,
                  pltpu.VMEM((3, d_model // 16, 16 * n_heads, e), _BF16))

    def prep_attn(vals):
        ha[_half((m2, vals.shape[0])), :] = _pack(_layernorm(vals))

    def prep_glu(buf, part, vals):
        h = _layernorm(vals)
        blocks = _lhs_blocks(h[:seg, :half], h[:seg, half:], h[seg:, :half], h[seg:, half:])
        for i, blk in enumerate(blocks):
            hb[buf, i, pl.ds(pl.multiple_of(part * (seg // 2), seg // 2), seg // 2), :] = _pack(blk)

    def finish_glu(buf, part, top, bottom):
        c11, c12, c21, c22 = _out_blocks(*(macc[buf, i, rows_of(part), :] for i in range(7)))
        z_top = (load_segs([top]) + jnp.concatenate([c11, c12], axis=1)).astype(_BF16)
        z_bot = (load_segs([bottom]) + jnp.concatenate([c21, c22], axis=1)).astype(_BF16)
        res[rows_of(top), :] = z_top
        res[rows_of(bottom), :] = z_bot
        return z_top

    def run(order, step=None, a_segs=(), layer=None, first=False, side=None):
        a_rows = m2 + len(a_segs) * seg
        if step is not None:
            part = step % 2
            buf = (step // 2) % 2
        qkv, probs, att, hid = {}, {}, {}, {}
        for op, i in order:
            if op == "ZFIN":
                done = jnp.where(step >= _LEAD, step - _LEAD, spare)
                z1 = finish_glu(1 - buf, part, step, done)
                prep_attn(jnp.concatenate(
                    [load_segs(a_segs[:1]), z1.astype(_F32)], axis=0))
            elif op == "SIDE":
                side(i)
            elif op == "QKV" and first and layer is not None:
                project_early(2, i)
                qkv[i] = [_unpack(early[w, i, _half((0, a_rows)), :]) for w in range(3)]
            elif op == "QKV" and first:
                rows = pl.ds(pl.multiple_of((m2 + (1 + step) * seg) // 2, 8), seg // 2)
                qkv[i] = [
                    jnp.concatenate([t[:m2], _unpack(early[w, i, rows, :]), t[m2:]], axis=0)
                    for w, t in enumerate(project(m2 + seg, i))]
            elif op == "QKV":
                qkv[i] = project(a_rows, i)
            elif op == "S":
                fill = bias2[...] if layer is None else bias1[layer]
                keep = fill > 0
                ps = []
                for h in range(_HG):
                    q = qkv[i][0][:, h * e:(h + 1) * e]
                    k = qkv[i][1][:, h * e:(h + 1) * e]
                    s = lax.dot_general(q, k, (((1,), (1,)), ((), ())),
                                        preferred_element_type=_F32)
                    s = jnp.where(keep, s * scale, fill)
                    p = jnp.exp(s - jnp.max(s, axis=-1, keepdims=True))
                    p = p / jnp.sum(p, axis=-1, keepdims=True)
                    ps.append(p.astype(_BF16))
                probs[i] = ps
            elif op == "PV":
                heads = []
                for h in range(_HG):
                    v = qkv[i][2][:, h * e:(h + 1) * e]
                    heads.append(_dot(probs[i][h], v).astype(_BF16))
                att[i] = jnp.concatenate(heads, axis=1)
            elif op == "O":
                if first and layer is not None:
                    wo_copy(i).wait()
                out = _dot(att[i], wo[pl.ds(i * _HG * e, _HG * e), :])
                if i == 0:
                    oacc[pl.ds(0, m2), :] = out[:m2]
                    oacc[pl.ds(m2, a_rows - m2), :] = load_segs(a_segs) + out[m2:]
                else:
                    oacc[pl.ds(0, a_rows), :] += out
            elif op == "YFIN":
                y = oacc[pl.ds(m2, a_rows - m2), :].astype(_BF16)
                for k, s in enumerate(a_segs):
                    res[rows_of(s), :] = y[k * seg:(k + 1) * seg]
                mem = oacc[pl.ds(0, m2), :]
                if layer is None:
                    prep_glu(1 - buf, part, y.astype(_F32))
                else:
                    row = lax.broadcasted_iota(jnp.int32, mem.shape, 0)
                    mine = (row >= layer * n_mem) & (row < (layer + 1) * n_mem)
                    mem = jnp.where(mine, mem, _unpack(ha[_half((0, m2)), :]).astype(_F32))
                ha[_half((0, m2)), :] = _pack(mem)
            elif op == "GU":
                c = part * n_c + i
                c11, c12, c21, c22 = _out_blocks(
                    *(_dot(_unpack(hb[buf, k]), _unpack(wgu[k, c])) for k in range(7)))
                hid[i] = [blk.astype(_BF16) for blk in _lhs_blocks(
                    *(_gelu(blk[:, :_T]) * blk[:, _T:] for blk in (c11, c12, c21, c22)))]
            elif op == "D":
                lo, hi = i
                rows = pl.ds(pl.multiple_of((part * n_c + lo) * (_T // 2), _T // 2),
                             (hi - lo) * (_T // 2))
                for k in range(7):
                    lhs = jnp.concatenate([hid[c][k] for c in range(lo, hi)], axis=1)
                    out = _dot(lhs, _unpack(wd[k, rows, :]))
                    if lo == 0:
                        macc[buf, k] = jnp.where(part == 0, out, macc[buf, k] + out)
                    else:
                        macc[buf, k] += out

    attn_all = _attn_order(n_g) + [("O", n_g - 1), ("YFIN", 0)]

    def attn_alone(layer, lo, hi):
        order = list(attn_all)
        order.insert(order.index(("QKV", n_g - 1)) + 1, ("SIDE", 0))
        prep_attn(load_segs([lo]))
        loop(lo, hi, lambda s: run(
            order, a_segs=[s], layer=layer,
            side=lambda _: prep_attn(load_segs([jnp.minimum(s + 1, hi - 1)]))))

    def head_start(raw_g, raw_u, raw_d):
        def raw_copy(w, c):
            start = c * 2 * _T
            cols = pl.ds(start if isinstance(c, int) else pl.multiple_of(start, 2 * _T), 2 * _T)
            src, dst = ((wg_hbm.at[:, cols], raw_g.at[c]), (wu_hbm.at[:, cols], raw_u.at[c]),
                        (wd_hbm.at[cols], raw_d.at[c]))[w]
            return pltpu.make_async_copy(src, dst, sem_f.at[w, c])

        def split(raw, c, r, dr, k, dk, store):
            quads = [pltpu.bitcast(raw[c, pl.ds(r + i * dr, 16), pl.ds(k + j * dk, _T)],
                                   jnp.uint32)
                     for i in range(2) for j in range(2)]
            even = _rhs_blocks(*(pltpu.bitcast(q << 16, _F32) for q in quads))
            odd = _rhs_blocks(
                *(pltpu.bitcast(q & jnp.uint32(0xFFFF0000), _F32) for q in quads))
            for i, pair in enumerate(zip(even, odd)):
                if i in (1, 4):
                    store(i, quads[0 if i == 1 else 3])
                else:
                    packed = pltpu.pack_elementwise(list(pair), packed_dtype=_BF16)
                    store(i, pltpu.bitcast(packed, jnp.uint32))

        def split_piece(c, n):
            w, n = divmod(n, half // 16)
            if w < 2:
                def store(i, val):
                    wgu[i, c, _half((n * 16, 16)), pl.ds(w * _T, _T)] = val
                split((raw_g, raw_u)[w], c, n * 16, half, 0, _T, store)
            else:
                r, k = divmod(n, half // _T)

                def store(i, val):
                    row = pl.multiple_of(c * (_T // 2) + r * 8, 8)
                    wd[i, pl.ds(row, 8), pl.ds(k * _T, _T)] = val
                split(raw_d, c, r * 16, _T, k * _T, half, store)

        def fetch():
            for c in range(n_chunks):
                for w in range(3):
                    raw_copy(w, c).start()

        def split_chunk(c):
            for w in range(3):
                raw_copy(w, c).wait()
            for n in range(3 * (half // 16)):
                split_piece(c, n)

        late = (_WINDOW + n_g) // 2
        for g in range(_WINDOW, late):
            wo_copy(g).start()
        order = list(attn_all)
        order.insert(order.index(("O", _FIRST_GLU_AT)) + 1, ("SIDE", 0))
        order.insert(order.index(("O", 0)) + 1, ("SIDE", 1))
        run(order, a_segs=[0], layer=0, first=True,
            side=lambda k: [wo_copy(g).start() for g in range(late, n_g)] if k else fetch())
        attn_alone(0, 1, _LEAD)
        x_copy(1).start()
        loop(0, n_chunks, split_chunk)

    pl.run_scoped(head_start,
                  pltpu.VMEM((n_chunks, d_model, 2 * _T), _BF16),
                  pltpu.VMEM((n_chunks, d_model, 2 * _T), _BF16),
                  pltpu.VMEM((n_chunks, 2 * _T, d_model), _BF16))

    macc[...] = jnp.zeros(macc.shape, _F32)
    loop(0, 2, lambda part: prep_glu(0, part, load_segs([2 + part, part])))
    loop(0, 2, lambda step: run(_glu_order(n_c), step=step))
    loop(0, 2, lambda part: finish_glu(0, part, spare, part))
    x_copy(1).wait()

    def attn_step(j):
        prep_attn(load_segs([j]))
        run(attn_all, step=j, a_segs=[j + _LEAD, j], first=True)

    loop(0, 2, attn_step)

    def out_copy(c):
        n = _OUT_CH * seg
        return pltpu.make_async_copy(
            res.at[pl.ds(c * n, n)], out_hbm.at[pl.ds(c * n, n)], sem_out.at[c])

    n_out = n_seg // _OUT_CH
    n_main = n_seg - _LEAD
    full = _full_order(n_g, n_c)

    def full_step(j):
        run(full, step=j, a_segs=[j + _LEAD, j])
        final = j + 1 - _LEAD

        @pl.when((final > 0) & (final % _OUT_CH == 0))
        def _():
            out_copy(final // _OUT_CH - 1).start()

    loop(2, n_main, full_step)

    buf = (n_main // 2) % 2
    loop(0, 2, lambda part: finish_glu(
        1 - buf, part, n_main + part, n_main - _LEAD + part))

    def drain(phase):
        bottom = n_main - 2 + 2 * phase
        loop(2 * buf, 2 * buf + 2, lambda step: run(_glu_order(n_c), step=step))
        loop(0, 2, lambda part: finish_glu(buf, part, n_main + 2 + part, bottom + part))

        @pl.when(phase == 0)
        def _():
            out_copy(n_out - 2).start()
            attn_alone(1, n_main, n_seg)
            loop(0, 2, lambda part: prep_glu(
                buf, part, load_segs([n_main + 2 + part, n_main + part])))

    loop(0, 2, drain)
    out_copy(n_out - 1).start()
    for c in range(n_out):
        out_copy(c).wait()


@jax.jit
def pallas_interleave_layers__memory_aug_recurrent_mem_tr__glu_gated_geglu__prompt_kernel(
    A_x: jax.Array,
    A_mem0: jax.Array,
    A_Wq: jax.Array,
    A_Wk: jax.Array,
    A_Wv: jax.Array,
    A_Wo: jax.Array,
    A_seg_len: jax.Array,
    B_x: jax.Array,
    B_w_gate: jax.Array,
    B_w_up: jax.Array,
    B_w_down: jax.Array,
):
    del B_x
    _, s_len, d_model = A_x.shape
    _, n_heads, e = A_Wq.shape
    n_mem = A_mem0.shape[1]
    d_ff = B_w_gate.shape[1]
    seg = A_seg_len if isinstance(A_seg_len, int) else min(32, s_len)
    rows = 2 * (n_mem + seg)
    rows_early = 2 * n_mem + 3 * seg
    n_g = n_heads // _HG

    def stage_view(w):
        return w.reshape(d_model // 16, 16 * n_heads, e)

    n_chunks = d_ff // (2 * _T)
    half = d_model // 2
    any_spec = pl.BlockSpec(memory_space=pl.ANY)
    out = pl.pallas_call(
        functools.partial(_kernel, n_heads=n_heads, n_mem=n_mem, seg=seg),
        out_shape=jax.ShapeDtypeStruct((s_len, d_model), _BF16),
        in_specs=[any_spec, pl.BlockSpec(memory_space=pltpu.VMEM)] + [any_spec] * 7,
        out_specs=any_spec,
        scratch_shapes=[
            pltpu.VMEM((n_g, half, _HG * e), jnp.uint32),
            pltpu.VMEM((n_g, half, _HG * e), jnp.uint32),
            pltpu.VMEM((n_g, half, _HG * e), jnp.uint32),
            pltpu.VMEM((n_heads * e, d_model), _BF16),
            pltpu.VMEM((7, n_chunks, half // 2, 2 * _T), jnp.uint32),
            pltpu.VMEM((7, n_chunks * _T // 2, half), jnp.uint32),
            pltpu.VMEM((s_len + seg, d_model), _BF16),
            pltpu.VMEM((rows // 2, d_model), jnp.uint32),
            pltpu.VMEM((rows_early // 2, d_model), jnp.uint32),
            pltpu.VMEM((3, n_g, rows_early // 2, _HG * e), jnp.uint32),
            pltpu.VMEM((rows, d_model), _F32),
            pltpu.VMEM((2, 7, seg, half), jnp.uint32),
            pltpu.VMEM((2, 7, 2 * seg, half), _F32),
            pltpu.VMEM((rows, rows), _F32),
            pltpu.VMEM((2, rows - seg, rows - seg), _F32),
            pltpu.SemaphoreType.DMA((3, d_model // _DCH)),
            pltpu.SemaphoreType.DMA((2,)),
            pltpu.SemaphoreType.DMA((n_g,)),
            pltpu.SemaphoreType.DMA((3, n_chunks)),
            pltpu.SemaphoreType.DMA((s_len // seg // _OUT_CH,)),
        ],
        compiler_params=pltpu.CompilerParams(vmem_limit_bytes=110 * 1024 * 1024),
    )(
        A_x.reshape(s_len, d_model).astype(_BF16),
        A_mem0.reshape(n_mem, d_model).astype(_BF16),
        stage_view(A_Wq).astype(_BF16), stage_view(A_Wk).astype(_BF16),
        stage_view(A_Wv).astype(_BF16),
        A_Wo.reshape(n_heads * e, d_model).astype(_BF16),
        B_w_gate.astype(_BF16), B_w_up.astype(_BF16), B_w_down.astype(_BF16),
    )
    return out.reshape(1, s_len, d_model).astype(A_x.dtype)
```

```python
import functools
import math

import jax
import jax.numpy as jnp
from jax import lax
import jax.experimental.pallas as pl
import jax.experimental.pallas.tpu as pltpu

_BF16 = jnp.bfloat16
_F32 = jnp.float32

_HG = 4
_T = 128
_DCH = 128
_OUT_CH = 4
_LEAD = 4
_WINDOW = 4
_D_BATCH = 3


def _layernorm(x):
    m = jnp.mean(x, axis=-1, keepdims=True)
    c = x - m
    v = jnp.mean(c * c, axis=-1, keepdims=True)
    return c * lax.rsqrt(v + 1e-5)


def _gelu(x):
    k = math.sqrt(2.0 / math.pi)
    return x * (0.5 * (1.0 + jnp.tanh(k * (x + 0.044715 * (x * x * x)))))


def _dot(a, b):
    return jnp.dot(a, b, preferred_element_type=_F32)


def _pack(x):
    return pltpu.bitcast(x.astype(_BF16), jnp.uint32)


def _unpack(words):
    return pltpu.bitcast(words, _BF16)


def _half(rows):
    return pl.ds(rows[0] // 2, rows[1] // 2)


def _lhs_blocks(a11, a12, a21, a22):
    return (a11 + a22, a21 + a22, a11, a22, a11 + a12, a21 - a11, a12 - a22)


def _rhs_blocks(b11, b12, b21, b22):
    return (b11 + b22, b11, b12 - b22, b21 - b11, b22, b11 + b12, b21 + b22)


def _out_blocks(m1, m2, m3, m4, m5, m6, m7):
    return (m1 + m4 - m5 + m7, m3 + m5, m2 + m4, m1 - m2 + m3 + m6)


def _attn_order(n_g, fill=()):
    order = []
    done = 0
    for g in range(n_g + 1):
        if g >= 1:
            order.append(("S", g - 1))
        if g >= 2:
            order.append(("O", g - 2))
        upto = (len(fill) * (g + 1)) // (n_g + 1)
        order.extend(fill[done:upto])
        done = upto
        if g < n_g:
            order.append(("QKV", g))
        if g >= 1:
            order.append(("PV", g - 1))
    return order


def _glu_order(n_c):
    order = []
    start = 0
    for c in range(n_c):
        order.append(("GU", c))
        if c - start == _D_BATCH and c < n_c - 1:
            order.append(("D", (start, c)))
            start = c
    if n_c - start > 1:
        order.append(("D", (start, n_c - 1)))
    order.append(("D", (n_c - 1, n_c)))
    return order


def _full_order(n_g, n_c):
    glu = _glu_order(n_c)
    return ([glu[0], ("ZFIN", 0)] + _attn_order(n_g, glu[1:-2])
            + [glu[-2], ("O", n_g - 1), ("YFIN", 0), glu[-1]])


def _kernel(x_hbm, mem0_ref, wq_hbm, wk_hbm, wv_hbm, wo_hbm, wg_hbm, wu_hbm, wd_hbm,
            out_hbm,
            wq, wk, wv, wo, wgu, wd, res, ha, h0, early, oacc, hb, macc, bias2, bias1,
            sem_stage, sem_x, sem_o, sem_f, sem_out, *, n_heads, n_mem, seg):
    s_len, d_model = x_hbm.shape
    d_ff = wg_hbm.shape[1]
    e = wo.shape[0] // n_heads
    n_seg = s_len // seg
    n_g = n_heads // _HG
    n_chunks = d_ff // (2 * _T)
    n_c = n_chunks // 2
    n_dch = d_model // _DCH
    half = d_model // 2
    m2 = 2 * n_mem
    scale = e ** -0.5
    spare = n_seg
    wqkv = (wq, wk, wv)

    x_head = (_LEAD + 2) * seg

    def x_copy(i):
        rows = pl.ds(0, x_head) if i == 0 else pl.ds(x_head, s_len - x_head)
        return pltpu.make_async_copy(x_hbm.at[rows], res.at[rows], sem_x.at[i])

    def wo_copy(g):
        rows = pl.ds(g * _HG * e, _HG * e)
        return pltpu.make_async_copy(wo_hbm.at[rows], wo.at[rows], sem_o.at[g])

    def rows_of(s):
        if isinstance(s, int):
            return pl.ds(s * seg, seg)
        return pl.ds(pl.multiple_of(s * seg, seg), seg)

    def load_segs(segs):
        return jnp.concatenate([res[rows_of(s), :] for s in segs], axis=0).astype(_F32)

    def loop(lo, hi, fn):
        def body(i, carry):
            fn(i)
            return carry
        lax.fori_loop(lo, hi, body, 0)

    def project_early(w, g):
        early[w, g] = _pack(_dot(_unpack(h0[...]), _unpack(wqkv[w][g])))

    def project(n_rows, g):
        h = _unpack(ha[_half((0, n_rows)), :])
        return [_dot(h, _unpack(w[g])).astype(_BF16) for w in wqkv]

    def load_attention_weights(stage):
        blk = _DCH // 16

        def stage_copy(w, c):
            start = c * blk if isinstance(c, int) else pl.multiple_of(c * blk, blk)
            return pltpu.make_async_copy(
                (wq_hbm, wk_hbm, wv_hbm)[w].at[pl.ds(start, blk)],
                stage.at[w, pl.ds(start, blk)], sem_stage.at[w, c])

        x_copy(0).start()
        for c in range(_WINDOW):
            stage_copy(0, c).start()

        def score_fill(n_rows, layer_of_token):
            r_id = lax.broadcasted_iota(jnp.int32, (n_rows, n_rows), 0)
            c_id = lax.broadcasted_iota(jnp.int32, (n_rows, n_rows), 1)

            def layer_of(i):
                return jnp.where(i < m2, i // n_mem, layer_of_token(i - m2))

            same = layer_of(r_id) == layer_of(c_id)
            keep = same & ((r_id < m2) | (r_id >= c_id))
            return jnp.where(keep, 1.0, jnp.where(same, -1e9, -jnp.inf)).astype(_F32)

        bias2[...] = score_fill(m2 + 2 * seg, lambda i: i // seg)
        for layer in range(2):
            bias1[layer] = score_fill(m2 + seg, lambda i, layer=layer: layer)
        res[pl.ds(spare * seg, seg), :] = jnp.zeros((seg, d_model), _BF16)
        x_copy(0).wait()
        mem0 = mem0_ref[...].astype(_F32)
        mem0 = _pack(jnp.concatenate([mem0, mem0], axis=0))
        ha[_half((0, m2)), :] = mem0
        h0[_half((0, m2)), :] = mem0
        for k, s in enumerate((0, _LEAD, _LEAD + 1)):
            h0[_half((m2 + k * seg, seg)), :] = _pack(_layernorm(load_segs([s])))

        for w in range(3):
            def relayout(i, w=w):
                d0 = pl.multiple_of(i * 8, 8)
                for part in range(n_heads // 16):
                    v = [pltpu.bitcast(stage[w, i, pl.ds(d * n_heads + part * 16, 16), :],
                                       jnp.uint32) for d in range(16)]
                    even = jnp.stack([(v[2 * p] & jnp.uint32(0xFFFF)) | (v[2 * p + 1] << 16)
                                      for p in range(8)])
                    odd = jnp.stack([(v[2 * p] >> 16) | (v[2 * p + 1] & jnp.uint32(0xFFFF0000))
                                     for p in range(8)])
                    for k, val in enumerate((even, odd)):
                        val = jnp.swapaxes(val, 0, 1)
                        for j in range(8):
                            h = 2 * (part * 8 + j) + k
                            wqkv[w][h // _HG, pl.ds(d0, 8), pl.ds((h % _HG) * e, e)] = val[j]

            def chunk(c, w=w, relayout=relayout):
                stage_copy(w, c).wait()

                @pl.when(c + _WINDOW < n_dch)
                def _():
                    stage_copy(w, c + _WINDOW).start()

                @pl.when(c + _WINDOW >= n_dch)
                def _():
                    nxt = c + _WINDOW - n_dch
                    (stage_copy(w + 1, nxt) if w < 2 else wo_copy(nxt)).start()

                loop(c * blk, (c + 1) * blk, relayout)
                if w > 0:
                    project_early(w - 1, c)

            loop(0, n_dch, chunk)

    pl.run_scoped(load_attention_weights,
                  pltpu.VMEM((3, d_model // 16, 16 * n_heads, e), _BF16))

    def prep_attn(vals):
        ha[_half((m2, vals.shape[0])), :] = _pack(_layernorm(vals))

    def prep_glu(buf, part, vals):
        h = _layernorm(vals)
        blocks = _lhs_blocks(h[:seg, :half], h[:seg, half:], h[seg:, :half], h[seg:, half:])
        for i, blk in enumerate(blocks):
            hb[buf, i, pl.ds(pl.multiple_of(part * (seg // 2), seg // 2), seg // 2), :] = _pack(blk)

    def finish_glu(buf, part, top, bottom):
        c11, c12, c21, c22 = _out_blocks(*(macc[buf, i, rows_of(part), :] for i in range(7)))
        z_top = (load_segs([top]) + jnp.concatenate([c11, c12], axis=1)).astype(_BF16)
        z_bot = (load_segs([bottom]) + jnp.concatenate([c21, c22], axis=1)).astype(_BF16)
        res[rows_of(top), :] = z_top
        res[rows_of(bottom), :] = z_bot
        return z_top

    def run(order, step=None, a_segs=(), layer=None, first=False, side=None):
        a_rows = m2 + len(a_segs) * seg
        if step is not None:
            part = step % 2
            buf = (step // 2) % 2
        qkv, probs, att, hid = {}, {}, {}, {}
        for op, i in order:
            if op == "ZFIN":
                done = jnp.where(step >= _LEAD, step - _LEAD, spare)
                z1 = finish_glu(1 - buf, part, step, done)
                prep_attn(jnp.concatenate(
                    [load_segs(a_segs[:1]), z1.astype(_F32)], axis=0))
            elif op == "SIDE":
                side(i)
            elif op == "QKV" and first and layer is not None:
                project_early(2, i)
                qkv[i] = [_unpack(early[w, i, _half((0, a_rows)), :]) for w in range(3)]
            elif op == "QKV" and first:
                rows = pl.ds(pl.multiple_of((m2 + (1 + step) * seg) // 2, 8), seg // 2)
                qkv[i] = [
                    jnp.concatenate([t[:m2], _unpack(early[w, i, rows, :]), t[m2:]], axis=0)
                    for w, t in enumerate(project(m2 + seg, i))]
            elif op == "QKV":
                qkv[i] = project(a_rows, i)
            elif op == "S":
                fill = bias2[...] if layer is None else bias1[layer]
                keep = fill > 0
                ps = []
                for h in range(_HG):
                    q = qkv[i][0][:, h * e:(h + 1) * e]
                    k = qkv[i][1][:, h * e:(h + 1) * e]
                    s = lax.dot_general(q, k, (((1,), (1,)), ((), ())),
                                        preferred_element_type=_F32)
                    s = jnp.where(keep, s * scale, fill)
                    p = jnp.exp(s - jnp.max(s, axis=-1, keepdims=True))
                    p = p / jnp.sum(p, axis=-1, keepdims=True)
                    ps.append(p.astype(_BF16))
                probs[i] = ps
            elif op == "PV":
                heads = []
                for h in range(_HG):
                    v = qkv[i][2][:, h * e:(h + 1) * e]
                    heads.append(_dot(probs[i][h], v).astype(_BF16))
                att[i] = jnp.concatenate(heads, axis=1)
            elif op == "O":
                if first and layer is not None:
                    wo_copy(i).wait()
                out = _dot(att[i], wo[pl.ds(i * _HG * e, _HG * e), :])
                if i == 0:
                    oacc[pl.ds(0, m2), :] = out[:m2]
                    oacc[pl.ds(m2, a_rows - m2), :] = load_segs(a_segs) + out[m2:]
                else:
                    oacc[pl.ds(0, a_rows), :] += out
            elif op == "YFIN":
                y = oacc[pl.ds(m2, a_rows - m2), :].astype(_BF16)
                for k, s in enumerate(a_segs):
                    res[rows_of(s), :] = y[k * seg:(k + 1) * seg]
                mem = oacc[pl.ds(0, m2), :]
                if layer is None:
                    prep_glu(1 - buf, part, y.astype(_F32))
                else:
                    row = lax.broadcasted_iota(jnp.int32, mem.shape, 0)
                    mine = (row >= layer * n_mem) & (row < (layer + 1) * n_mem)
                    mem = jnp.where(mine, mem, _unpack(ha[_half((0, m2)), :]).astype(_F32))
                ha[_half((0, m2)), :] = _pack(mem)
            elif op == "GU":
                c = part * n_c + i
                c11, c12, c21, c22 = _out_blocks(
                    *(_dot(_unpack(hb[buf, k]), _unpack(wgu[k, c])) for k in range(7)))
                hid[i] = [blk.astype(_BF16) for blk in _lhs_blocks(
                    *(_gelu(blk[:, :_T]) * blk[:, _T:] for blk in (c11, c12, c21, c22)))]
            elif op == "D":
                lo, hi = i
                rows = pl.ds(pl.multiple_of((part * n_c + lo) * (_T // 2), _T // 2),
                             (hi - lo) * (_T // 2))
                for k in range(7):
                    lhs = jnp.concatenate([hid[c][k] for c in range(lo, hi)], axis=1)
                    out = _dot(lhs, _unpack(wd[k, rows, :]))
                    if lo == 0:
                        macc[buf, k] = jnp.where(part == 0, out, macc[buf, k] + out)
                    else:
                        macc[buf, k] += out

    attn_all = _attn_order(n_g) + [("O", n_g - 1), ("YFIN", 0)]

    def attn_alone(layer, lo, hi):
        order = list(attn_all)
        order.insert(order.index(("QKV", n_g - 1)) + 1, ("SIDE", 0))
        prep_attn(load_segs([lo]))
        loop(lo, hi, lambda s: run(
            order, a_segs=[s], layer=layer,
            side=lambda _: prep_attn(load_segs([jnp.minimum(s + 1, hi - 1)]))))

    def head_start(raw_g, raw_u, raw_d):
        def raw_copy(w, c):
            start = c * 2 * _T
            cols = pl.ds(start if isinstance(c, int) else pl.multiple_of(start, 2 * _T), 2 * _T)
            src, dst = ((wg_hbm.at[:, cols], raw_g.at[c]), (wu_hbm.at[:, cols], raw_u.at[c]),
                        (wd_hbm.at[cols], raw_d.at[c]))[w]
            return pltpu.make_async_copy(src, dst, sem_f.at[w, c])

        def split(raw, c, r, dr, k, dk, store):
            quads = [pltpu.bitcast(raw[c, pl.ds(r + i * dr, 16), pl.ds(k + j * dk, _T)],
                                   jnp.uint32)
                     for i in range(2) for j in range(2)]
            even = _rhs_blocks(*(pltpu.bitcast(q << 16, _F32) for q in quads))
            odd = _rhs_blocks(
                *(pltpu.bitcast(q & jnp.uint32(0xFFFF0000), _F32) for q in quads))
            for i, pair in enumerate(zip(even, odd)):
                if i in (1, 4):
                    store(i, quads[0 if i == 1 else 3])
                else:
                    packed = pltpu.pack_elementwise(list(pair), packed_dtype=_BF16)
                    store(i, pltpu.bitcast(packed, jnp.uint32))

        def split_piece(c, n):
            w, n = divmod(n, half // 16)
            if w < 2:
                def store(i, val):
                    wgu[i, c, _half((n * 16, 16)), pl.ds(w * _T, _T)] = val
                split((raw_g, raw_u)[w], c, n * 16, half, 0, _T, store)
            else:
                r, k = divmod(n, half // _T)

                def store(i, val):
                    row = pl.multiple_of(c * (_T // 2) + r * 8, 8)
                    wd[i, pl.ds(row, 8), pl.ds(k * _T, _T)] = val
                split(raw_d, c, r * 16, _T, k * _T, half, store)

        def split_chunk(c):
            for w in range(3):
                raw_copy(w, c).wait()
            for n in range(3 * (half // 16)):
                split_piece(c, n)

        late = (_WINDOW + n_g) // 2

        def fetch_more(k):
            if k == 0:
                for g in range(late, n_g):
                    wo_copy(g).start()
            else:
                for c in range(n_chunks):
                    for w in range(3):
                        raw_copy(w, c).start()

        for g in range(_WINDOW, late):
            wo_copy(g).start()
        order = list(attn_all)
        for k, g in enumerate((0, n_g // 2)):
            order.insert(order.index(("O", g)) + 1, ("SIDE", k))
        run(order, a_segs=[0], layer=0, first=True, side=fetch_more)
        attn_alone(0, 1, _LEAD)
        x_copy(1).start()
        loop(0, n_chunks, split_chunk)

    pl.run_scoped(head_start,
                  pltpu.VMEM((n_chunks, d_model, 2 * _T), _BF16),
                  pltpu.VMEM((n_chunks, d_model, 2 * _T), _BF16),
                  pltpu.VMEM((n_chunks, 2 * _T, d_model), _BF16))

    macc[...] = jnp.zeros(macc.shape, _F32)
    loop(0, 2, lambda part: prep_glu(0, part, load_segs([2 + part, part])))
    loop(0, 2, lambda step: run(_glu_order(n_c), step=step))
    loop(0, 2, lambda part: finish_glu(0, part, spare, part))
    x_copy(1).wait()

    def attn_step(j):
        prep_attn(load_segs([j]))
        run(attn_all, step=j, a_segs=[j + _LEAD, j], first=True)

    loop(0, 2, attn_step)

    def out_copy(c):
        n = _OUT_CH * seg
        return pltpu.make_async_copy(
            res.at[pl.ds(c * n, n)], out_hbm.at[pl.ds(c * n, n)], sem_out.at[c])

    n_out = n_seg // _OUT_CH
    n_main = n_seg - _LEAD
    full = _full_order(n_g, n_c)

    def full_step(j):
        run(full, step=j, a_segs=[j + _LEAD, j])
        final = j + 1 - _LEAD

        @pl.when((final > 0) & (final % _OUT_CH == 0))
        def _():
            out_copy(final // _OUT_CH - 1).start()

    loop(2, n_main, full_step)

    buf = (n_main // 2) % 2
    loop(0, 2, lambda part: finish_glu(
        1 - buf, part, n_main + part, n_main - _LEAD + part))

    def drain(phase):
        bottom = n_main - 2 + 2 * phase
        loop(2 * buf, 2 * buf + 2, lambda step: run(_glu_order(n_c), step=step))
        loop(0, 2, lambda part: finish_glu(buf, part, n_main + 2 + part, bottom + part))

        @pl.when(phase == 0)
        def _():
            out_copy(n_out - 2).start()
            attn_alone(1, n_main, n_seg)
            loop(0, 2, lambda part: prep_glu(
                buf, part, load_segs([n_main + 2 + part, n_main + part])))

    loop(0, 2, drain)
    out_copy(n_out - 1).start()
    for c in range(n_out):
        out_copy(c).wait()


@jax.jit
def pallas_interleave_layers__memory_aug_recurrent_mem_tr__glu_gated_geglu__prompt_kernel(
    A_x: jax.Array,
    A_mem0: jax.Array,
    A_Wq: jax.Array,
    A_Wk: jax.Array,
    A_Wv: jax.Array,
    A_Wo: jax.Array,
    A_seg_len: jax.Array,
    B_x: jax.Array,
    B_w_gate: jax.Array,
    B_w_up: jax.Array,
    B_w_down: jax.Array,
):
    del B_x
    _, s_len, d_model = A_x.shape
    _, n_heads, e = A_Wq.shape
    n_mem = A_mem0.shape[1]
    d_ff = B_w_gate.shape[1]
    seg = A_seg_len if isinstance(A_seg_len, int) else min(32, s_len)
    rows = 2 * (n_mem + seg)
    rows_early = 2 * n_mem + 3 * seg
    n_g = n_heads // _HG

    def stage_view(w):
        return w.reshape(d_model // 16, 16 * n_heads, e)

    n_chunks = d_ff // (2 * _T)
    half = d_model // 2
    any_spec = pl.BlockSpec(memory_space=pl.ANY)
    out = pl.pallas_call(
        functools.partial(_kernel, n_heads=n_heads, n_mem=n_mem, seg=seg),
        out_shape=jax.ShapeDtypeStruct((s_len, d_model), _BF16),
        in_specs=[any_spec, pl.BlockSpec(memory_space=pltpu.VMEM)] + [any_spec] * 7,
        out_specs=any_spec,
        scratch_shapes=[
            pltpu.VMEM((n_g, half, _HG * e), jnp.uint32),
            pltpu.VMEM((n_g, half, _HG * e), jnp.uint32),
            pltpu.VMEM((n_g, half, _HG * e), jnp.uint32),
            pltpu.VMEM((n_heads * e, d_model), _BF16),
            pltpu.VMEM((7, n_chunks, half // 2, 2 * _T), jnp.uint32),
            pltpu.VMEM((7, n_chunks * _T // 2, half), jnp.uint32),
            pltpu.VMEM((s_len + seg, d_model), _BF16),
            pltpu.VMEM((rows // 2, d_model), jnp.uint32),
            pltpu.VMEM((rows_early // 2, d_model), jnp.uint32),
            pltpu.VMEM((3, n_g, rows_early // 2, _HG * e), jnp.uint32),
            pltpu.VMEM((rows, d_model), _F32),
            pltpu.VMEM((2, 7, seg, half), jnp.uint32),
            pltpu.VMEM((2, 7, 2 * seg, half), _F32),
            pltpu.VMEM((rows, rows), _F32),
            pltpu.VMEM((2, rows - seg, rows - seg), _F32),
            pltpu.SemaphoreType.DMA((3, d_model // _DCH)),
            pltpu.SemaphoreType.DMA((2,)),
            pltpu.SemaphoreType.DMA((n_g,)),
            pltpu.SemaphoreType.DMA((3, n_chunks)),
            pltpu.SemaphoreType.DMA((s_len // seg // _OUT_CH,)),
        ],
        compiler_params=pltpu.CompilerParams(vmem_limit_bytes=110 * 1024 * 1024),
    )(
        A_x.reshape(s_len, d_model).astype(_BF16),
        A_mem0.reshape(n_mem, d_model).astype(_BF16),
        stage_view(A_Wq).astype(_BF16), stage_view(A_Wk).astype(_BF16),
        stage_view(A_Wv).astype(_BF16),
        A_Wo.reshape(n_heads * e, d_model).astype(_BF16),
        B_w_gate.astype(_BF16), B_w_up.astype(_BF16), B_w_down.astype(_BF16),
    )
    return out.reshape(1, s_len, d_model).astype(A_x.dtype)
```
